```python
import jax
import jax.numpy as jnp

def _softmax(x, axis=-1):
    return jax.nn.softmax(x, axis=axis)

def _gelu(x):
    return jax.nn.gelu(x, approximate=True)

def _silu(x):
    return jax.nn.silu(x)

def _sigmoid(x):
    return jax.nn.sigmoid(x)

def _layernorm(x, axis=-1, eps=1e-05):
    m = jnp.mean(x, axis=axis, keepdims=True)
    v = jnp.var(x, axis=axis, keepdims=True)
    return (x - m) / jnp.sqrt(v + eps)

def _scatter_add(tgt, idx, src, axis=0):
    return tgt.at[idx].add(src)

def _segment_sum(src, seg, n):
    return jax.ops.segment_sum(src, seg, n)

class _Rng:

    def __init__(self, key):
        self._k = key

    def _next(self):
        self._k, sub = jax.random.split(self._k)
        return sub

    def normal(self, shape):
        return jax.random.normal(self._next(), shape, dtype=jnp.bfloat16)

    def randint(self, lo, hi, shape):
        return jax.random.randint(self._next(), shape, lo, hi, dtype=jnp.int32)

    def uniform(self, shape, lo=0.0, hi=1.0):
        return jax.random.uniform(self._next(), shape, jnp.bfloat16, lo, hi)

    def permutation(self, n):
        return jax.random.permutation(self._next(), n)
kernel_name = 'interleave_layers__memory_aug_recurrent_mem_tr__spectral_gfnet__prompt'

def setup_inputs():
    _rng = _Rng(jax.random.key(int.from_bytes(__import__("os").urandom(4), "little")))
    _w = lambda a: (lambda t: t.astype(jnp.bfloat16) if jnp.issubdtype(t.dtype, jnp.floating) else t)(jnp.asarray(a))

    def _A_setup():
        B, S, Dm = (1, 2048, 640)
        H, Dh = (32, 128)
        M, seg = (8, 32)
        seg = min(seg, S)
        S = S // seg * seg
        return {'x': _w((lambda *s: _rng.normal(s) * 0.05)(B, S, Dm)), 'mem0': _w((lambda *s: _rng.normal(s) * 0.05)(B, M, Dm)), 'Wq': _w((lambda *s: _rng.normal(s) * 0.05)(Dm, H, Dh) * Dm ** (-0.5)), 'Wk': _w((lambda *s: _rng.normal(s) * 0.05)(Dm, H, Dh) * Dm ** (-0.5)), 'Wv': _w((lambda *s: _rng.normal(s) * 0.05)(Dm, H, Dh) * Dm ** (-0.5)), 'Wo': _w((lambda *s: _rng.normal(s) * 0.05)(H, Dh, Dm) * (H * Dh) ** (-0.5)), 'seg_len': seg}
    _A_in = _A_setup()

    def _B_setup():
        B, S, D = (1, 2048, 640)
        Df = D // 2 + 1
        return {'x': _w((lambda *s: _rng.normal(s) * 0.05)(B, S, D)), 'w_r': _w((lambda *s: _rng.normal(s) * 0.05)(S, Df) * 0.02), 'w_i': _w((lambda *s: _rng.normal(s) * 0.05)(S, Df) * 0.02)}
    _B_in = _B_setup()
    return {'A_x': _A_in['x'], 'A_mem0': _A_in['mem0'], 'A_Wq': _A_in['Wq'], 'A_Wk': _A_in['Wk'], 'A_Wv': _A_in['Wv'], 'A_Wo': _A_in['Wo'], 'A_seg_len': _A_in['seg_len'], 'B_x': _B_in['x'], 'B_w_r': _B_in['w_r'], 'B_w_i': _B_in['w_i']}

def reference(A_x, A_mem0, A_Wq, A_Wk, A_Wv, A_Wo, A_seg_len, B_x, B_w_r, B_w_i):

    def _A_ref(x, mem0, Wq, Wk, Wv, Wo, seg_len):
        B, S, Dm = x.shape
        H, Dh = (Wq.shape[1], Wq.shape[2])
        M = mem0.shape[1]
        scale = Dh ** (-0.5)
        n_seg = S // seg_len
        L = M + seg_len
        idx = jnp.arange(L)
        mask = (idx[:, None] < M) | (idx[:, None] >= idx[None, :])
        mem = mem0
        outs = []
        for s in range(n_seg):
            xs = x[:, s * seg_len:(s + 1) * seg_len, :].copy()
            h = jnp.concatenate([mem, xs], axis=1)
            q = jnp.einsum('btd,dhe->bhte', h, Wq)
            k = jnp.einsum('btd,dhe->bhte', h, Wk)
            v = jnp.einsum('btd,dhe->bhte', h, Wv)
            scores = jnp.einsum('bhqe,bhke->bhqk', q, k) * scale
            scores = jnp.where(mask[None, None], scores, -1000000000.0)
            p = _softmax(scores, axis=-1)
            o = jnp.einsum('bhqk,bhke->bhqe', p, v)
            o = jnp.einsum('bhte,hed->btd', o, Wo)
            mem = o[:, :M, :].copy()
            outs.append(o[:, M:, :])
        return jnp.concatenate(outs, axis=1)

    def _B_ref(x, w_r, w_i):
        B, S, D = x.shape
        X = (lambda x, axes=(-2, -1): jnp.fft.rfft2(x.astype(jnp.float32), axes=axes))(x, axes=(-2, -1))
        W = w_r + 1j * w_i
        X = X * W
        y = (lambda x, s, axes=(-2, -1): jnp.fft.irfft2(x, s=s, axes=axes).astype(jnp.bfloat16))(X, (S, D), axes=(-2, -1))
        return y
    x = A_x
    x = x + _A_ref(_layernorm(x, axis=-1), A_mem0, A_Wq, A_Wk, A_Wv, A_Wo, A_seg_len)
    x = x + _B_ref(_layernorm(x, axis=-1), B_w_r, B_w_i)
    x = x + _A_ref(_layernorm(x, axis=-1), A_mem0, A_Wq, A_Wk, A_Wv, A_Wo, A_seg_len)
    x = x + _B_ref(_layernorm(x, axis=-1), B_w_r, B_w_i)
    return x
```

```python
import functools
import math

import jax
import jax.numpy as jnp
import numpy as np
import jax.experimental.pallas as pl
import jax.experimental.pallas.tpu as pltpu

F32 = jnp.float32
BF16 = jnp.bfloat16
LANES = 128
RADIX = 16
GROUP = 4
EPS = 1e-5
NEG = -1000000000.0


def _dft_constants(S, D):
    Df = D // 2 + 1
    P = -(-Df // LANES) * LANES
    nb = S // RADIX
    d = np.arange(D)[:, None]
    k = np.arange(Df)[None, :]
    ang = 2.0 * np.pi * ((d * k) % D) / D
    fwd_d = np.zeros((D, 2 * P))
    fwd_d[:, :Df] = np.cos(ang)
    fwd_d[:, P:P + Df] = -np.sin(ang)
    c = np.full((Df,), 2.0)
    c[0] = 1.0
    s = c.copy()
    s[0] = 0.0
    if D % 2 == 0:
        c[-1] = 1.0
        s[-1] = 0.0
    inv_d = np.zeros((2 * P, D))
    inv_d[:Df] = (np.cos(ang) * c / D).T
    inv_d[P:P + Df] = (-np.sin(ang) * s / D).T
    b = np.arange(nb)[None, None, :]
    f = np.arange(RADIX)[:, None, None] + RADIX * np.arange(nb)[None, :, None]
    ang = 2.0 * np.pi * ((b * f) % S) / S
    tr, ti = np.cos(ang), -np.sin(ang)
    fwd_s = np.concatenate([np.concatenate([tr, -ti], 2),
                            np.concatenate([ti, tr], 2)], 1)
    inv_s = np.swapaxes(fwd_s, 1, 2) / S
    return [a.astype(np.float32) for a in (fwd_d, inv_d, fwd_s, inv_s)]


def _fft(vals, sign):
    n = len(vals)
    if n == 1:
        return vals
    ev, od = _fft(vals[0::2], sign), _fft(vals[1::2], sign)
    lo, hi = [], []
    for j in range(n // 2):
        (er, ei), (pr, pi) = ev[j], od[j]
        if 4 * j == n:
            if sign > 0:
                lo.append((er - pi, ei + pr))
                hi.append((er + pi, ei - pr))
            else:
                lo.append((er + pi, ei - pr))
                hi.append((er - pi, ei + pr))
            continue
        if j > 0:
            c = math.cos(2 * math.pi * j / n)
            s = sign * math.sin(2 * math.pi * j / n)
            if 8 * j == n:
                pr, pi = ((pr - pi) * c, (pr + pi) * c) if sign > 0 else (
                    (pr + pi) * c, (pi - pr) * c)
            elif 8 * j == 3 * n:
                pr, pi = ((pr + pi) * c, (pi - pr) * c) if sign > 0 else (
                    (pr - pi) * c, (pr + pi) * c)
            else:
                pr, pi = pr * c - pi * s, pr * s + pi * c
        lo.append((er + pr, ei + pi))
        hi.append((er - pr, ei - pi))
    return lo + hi


def _dot(a, b):
    return jax.lax.dot_general(a, b, (((1,), (0,)), ((), ())),
                               preferred_element_type=F32)


def _dot_t(a, b):
    return jax.lax.dot_general(a, b, (((1,), (1,)), ((), ())),
                               preferred_element_type=F32)


def _layernorm(x):
    xc = x - jnp.mean(x, axis=-1, keepdims=True)
    var = jnp.mean(xc * xc, axis=-1, keepdims=True)
    return xc * jax.lax.rsqrt(var + EPS)


def _round(x):
    return x.astype(BF16).astype(F32)


def _kernel(x_hbm, mem_hbm, wq_hbm, wk_hbm, wv_hbm, wo_hbm, wr_hbm, wi_hbm,
            fd_hbm, id_hbm, fs_hbm, is_hbm, o_hbm,
            xb, memb, stage, w, wo, wrb, wib, fd, idm, fs, ism,
            x, h, u, filt, sems, *, S, D, H, Dh, M, seg):
    L = M + seg
    n_seg = S // seg
    nb = S // RADIX
    nc = u.shape[0] // 2
    P = nc * LANES
    Df = wrb.shape[1]
    HD = H * Dh
    n_chunk = D // LANES
    scale = Dh ** -0.5

    def get(r, c0, n):
        return jnp.concatenate([u[c0 + c, r, :] for c in range(n)], axis=1)

    def put(r, c0, val):
        for c in range(val.shape[1] // LANES):
            u[c0 + c, r, :] = val[:, c * LANES:(c + 1) * LANES]

    small = [(x_hbm, xb), (mem_hbm, memb), (wr_hbm, wrb), (wi_hbm, wib)]
    late = [(wo_hbm, wo), (fd_hbm, fd), (fs_hbm, fs), (is_hbm, ism),
            (id_hbm, idm)]
    copies = [pltpu.make_async_copy(s_, d_, sems.at[i])
              for i, (s_, d_) in enumerate(small + late)]
    base = len(copies)
    w_copies = []
    for t, src in enumerate((wq_hbm, wk_hbm, wv_hbm)):
        for c in range(n_chunk):
            i = t * n_chunk + c
            w_copies.append(pltpu.make_async_copy(
                src.at[pl.ds(c * LANES * H, LANES * H)], stage.at[i],
                sems.at[base + i]))
    for cp in copies[:len(small)] + w_copies + copies[len(small):]:
        cp.start()

    copies[0].wait()

    @pl.loop(0, S // LANES)
    def _(i):
        r = pl.ds(pl.multiple_of(i * LANES, LANES), LANES)
        xv = xb[r, :].astype(F32)
        x[r, :] = xv
        h[r, :] = _layernorm(xv)

    copies[2].wait()
    copies[3].wait()

    @pl.loop(0, S // LANES)
    def _(i):
        r = pl.ds(pl.multiple_of(i * LANES, LANES), LANES)
        z = jnp.zeros((LANES, P - Df), F32)
        put(r, 0, jnp.concatenate(
            [wrb[r, :].astype(F32), z, wib[r, :].astype(F32), z], axis=1))

    for f1 in range(RADIX):
        filt[f1] = get(pl.ds(f1, nb, stride=RADIX), 0, 2 * nc)

    stage32 = stage.bitcast(jnp.uint32)
    for i, cp in enumerate(w_copies):
        cp.wait()
        t, c = divmod(i, n_chunk)
        for j in range(H // 2):
            a = stage32[i, pl.ds(j, LANES // 2, stride=H), :]
            b = stage32[i, pl.ds(j + H // 2, LANES // 2, stride=H), :]
            even = (a & jnp.uint32(0xFFFF)) | (b << 16)
            odd = (a >> 16) | (b & jnp.uint32(0xFFFF0000))
            col = t * HD + 2 * j * Dh
            rows = pl.ds(c * LANES, LANES)
            w[rows, col:col + Dh] = pltpu.bitcast(even, BF16)
            w[rows, col + Dh:col + 2 * Dh] = pltpu.bitcast(odd, BF16)

    copies[1].wait()
    for cp in copies[len(small):]:
        cp.wait()

    n_grp = H // GROUP
    gw = GROUP * Dh

    def segment(s, mem):
        r = pl.ds(pl.multiple_of(s * seg, seg), seg)
        hs = jnp.concatenate([mem, h[r, :]], axis=0)
        row = jax.lax.broadcasted_iota(jnp.int32, (L, L), 0)
        col = jax.lax.broadcasted_iota(jnp.int32, (L, L), 1)
        mask = (row < M) | (row >= col)

        def project(g):
            q, k, v = [_dot(hs, w[:, t * HD + g * gw:t * HD + (g + 1) * gw])
                       for t in range(3)]
            return q, k.astype(BF16), v.astype(BF16)

        def probs(q, k):
            out = []
            for j in range(GROUP):
                c = slice(j * Dh, (j + 1) * Dh)
                sc = jnp.where(mask, _dot_t(q[:, c], k[:, c]) * scale, NEG)
                e = jnp.exp(sc - jnp.max(sc, axis=-1, keepdims=True))
                out.append((e, 1.0 / jnp.sum(e, axis=-1, keepdims=True)))
            return out

        def attend(ps, v):
            return jnp.concatenate(
                [_dot(e, v[:, j * Dh:(j + 1) * Dh]) * inv
                 for j, (e, inv) in enumerate(ps)], axis=1)

        qkv, ps, os_ = {}, {}, {}
        acc = None
        for t in range(n_grp + 3):
            if t < n_grp:
                qkv[t] = project(t)
            if 0 <= t - 1 < n_grp:
                ps[t - 1] = probs(qkv[t - 1][0], qkv[t - 1][1])
            if 0 <= t - 2 < n_grp:
                os_[t - 2] = attend(ps[t - 2], qkv[t - 2][2])
            if 0 <= t - 3 < n_grp:
                g = t - 3
                y = _dot(os_[g], wo[g * gw:(g + 1) * gw, :])
                acc = y if acc is None else acc + y
        xn = _round(x[r, :] + _round(acc[M:]))
        x[r, :] = xn
        h[r, :] = _layernorm(xn)
        return acc[:M]

    def butterflies(sign):
        @pl.loop(0, nb // 8)
        def _(i):
            for c in range(nc):
                rows = [pl.ds(pl.multiple_of(a * nb + i * 8, 8), 8)
                        for a in range(RADIX)]
                out = _fft([(u[c, r, :], u[nc + c, r, :]) for r in rows], sign)
                for r, (vr, vi) in zip(rows, out):
                    u[c, r, :] = vr
                    u[nc + c, r, :] = vi

    def spectral():
        blk = 256

        @pl.loop(0, S // blk)
        def _(i):
            r = pl.ds(pl.multiple_of(i * blk, blk), blk)
            put(r, 0, _dot(h[r, :], fd[...]))

        butterflies(-1)

        @pl.loop(0, RADIX)
        def _(f1):
            r = pl.ds(pl.multiple_of(f1 * nb, nb), nb)
            z = jnp.concatenate([get(r, 0, nc), get(r, nc, nc)],
                                axis=0).astype(BF16)
            y = _dot(fs[f1], z)
            yr, yi = y[:nb], y[nb:]
            wr, wi = filt[f1, :, :P], filt[f1, :, P:]
            z = jnp.concatenate([yr * wr - yi * wi, yr * wi + yi * wr],
                                axis=0).astype(BF16)
            y = _dot(ism[f1], z)
            put(r, 0, y[:nb])
            put(r, nc, y[nb:])

        butterflies(1)

        @pl.loop(0, S // blk)
        def _(i):
            r = pl.ds(pl.multiple_of(i * blk, blk), blk)
            y = _dot(get(r, 0, 2 * nc), idm[...])
            xn = _round(x[r, :] + _round(y))
            x[r, :] = xn
            h[r, :] = _layernorm(xn)

    @pl.loop(0, 2)
    def _(layer):
        jax.lax.fori_loop(0, n_seg, segment, memb[...].astype(F32))
        spectral()

    xb[...] = x[...].astype(BF16)
    pltpu.sync_copy(xb, o_hbm)


@functools.partial(jax.jit, static_argnames=("A_seg_len",))
def pallas_interleave_layers__memory_aug_recurrent_mem_tr__spectral_gfnet__prompt_kernel(
    A_x, A_mem0, A_Wq, A_Wk, A_Wv, A_Wo, A_seg_len, B_x, B_w_r, B_w_i,
):
    del B_x
    B, S, D = A_x.shape
    _, H, Dh = A_Wq.shape
    M = A_mem0.shape[1]
    assert B == 1 and Dh == LANES and S == RADIX * LANES and D % LANES == 0
    consts = [c.astype(BF16) for c in _dft_constants(S, D)]
    P2 = consts[0].shape[1]
    n_w = 3 * (D // LANES)
    args = [A_x.reshape(S, D), A_mem0.reshape(M, D),
            A_Wq.reshape(D * H, Dh), A_Wk.reshape(D * H, Dh),
            A_Wv.reshape(D * H, Dh), A_Wo.reshape(H * Dh, D),
            B_w_r, B_w_i] + consts
    out = pl.pallas_call(
        functools.partial(_kernel, S=S, D=D, H=H, Dh=Dh, M=M, seg=A_seg_len),
        out_shape=jax.ShapeDtypeStruct((S, D), BF16),
        in_specs=[pl.BlockSpec(memory_space=pl.ANY)] * len(args),
        out_specs=pl.BlockSpec(memory_space=pl.ANY),
        scratch_shapes=[
            pltpu.VMEM((S, D), BF16),
            pltpu.VMEM((M, D), BF16),
            pltpu.VMEM((n_w, LANES * H, Dh), BF16),
            pltpu.VMEM((D, 3 * H * Dh), BF16),
            pltpu.VMEM((H * Dh, D), BF16),
            pltpu.VMEM(B_w_r.shape, BF16),
            pltpu.VMEM(B_w_i.shape, BF16),
        ] + [pltpu.VMEM(c.shape, BF16) for c in consts] + [
            pltpu.VMEM((S, D), F32),
            pltpu.VMEM((S, D), F32),
            pltpu.VMEM((P2 // LANES, S, LANES), F32),
            pltpu.VMEM((RADIX, S // RADIX, P2), F32),
            pltpu.SemaphoreType.DMA((9 + n_w,)),
        ],
        compiler_params=pltpu.CompilerParams(vmem_limit_bytes=100 * 2 ** 20),
    )(*args)
    return out.reshape(B, S, D)
```

```python
import functools
import math

import jax
import jax.numpy as jnp
import numpy as np
import jax.experimental.pallas as pl
import jax.experimental.pallas.tpu as pltpu

F32 = jnp.float32
BF16 = jnp.bfloat16
LANES = 128
RADIX = 16
GROUP = 4
EPS = 1e-5
NEG = -1000000000.0


def _dft_constants(S, D):
    Df = D // 2 + 1
    P = -(-Df // LANES) * LANES
    nb = S // RADIX
    d = np.arange(D)[:, None]
    k = np.arange(Df)[None, :]
    ang = 2.0 * np.pi * ((d * k) % D) / D
    fwd_d = np.zeros((D, 2 * P))
    fwd_d[:, :Df] = np.cos(ang)
    fwd_d[:, P:P + Df] = -np.sin(ang)
    c = np.full((Df,), 2.0)
    c[0] = 1.0
    s = c.copy()
    s[0] = 0.0
    if D % 2 == 0:
        c[-1] = 1.0
        s[-1] = 0.0
    inv_d = np.zeros((2 * P, D))
    inv_d[:Df] = (np.cos(ang) * c / D).T
    inv_d[P:P + Df] = (-np.sin(ang) * s / D).T
    b = np.arange(nb)[None, None, :]
    f = np.arange(RADIX)[:, None, None] + RADIX * np.arange(nb)[None, :, None]
    ang = 2.0 * np.pi * ((b * f) % S) / S
    tr, ti = np.cos(ang), -np.sin(ang)
    fwd_s = np.concatenate([np.concatenate([tr, -ti], 2),
                            np.concatenate([ti, tr], 2)], 1)
    inv_s = np.swapaxes(fwd_s, 1, 2) / S
    return [a.astype(np.float32) for a in (fwd_d, inv_d, fwd_s, inv_s)]


def _fft(vals, sign):
    n = len(vals)
    if n == 1:
        return vals
    ev, od = _fft(vals[0::2], sign), _fft(vals[1::2], sign)
    lo, hi = [], []
    for j in range(n // 2):
        (er, ei), (pr, pi) = ev[j], od[j]
        if 4 * j == n:
            if sign > 0:
                lo.append((er - pi, ei + pr))
                hi.append((er + pi, ei - pr))
            else:
                lo.append((er + pi, ei - pr))
                hi.append((er - pi, ei + pr))
            continue
        if j > 0:
            c = math.cos(2 * math.pi * j / n)
            s = sign * math.sin(2 * math.pi * j / n)
            if 8 * j == n:
                pr, pi = ((pr - pi) * c, (pr + pi) * c) if sign > 0 else (
                    (pr + pi) * c, (pi - pr) * c)
            elif 8 * j == 3 * n:
                pr, pi = ((pr + pi) * c, (pi - pr) * c) if sign > 0 else (
                    (pr - pi) * c, (pr + pi) * c)
            else:
                pr, pi = pr * c - pi * s, pr * s + pi * c
        lo.append((er + pr, ei + pi))
        hi.append((er - pr, ei - pi))
    return lo + hi


def _dot(a, b):
    return jax.lax.dot_general(a, b, (((1,), (0,)), ((), ())),
                               preferred_element_type=F32)


def _dot_t(a, b):
    return jax.lax.dot_general(a, b, (((1,), (1,)), ((), ())),
                               preferred_element_type=F32)


def _unpack(tiles):
    return pltpu.bitcast(jnp.concatenate(tiles, axis=1), BF16)


def _layernorm(x):
    xc = x - jnp.mean(x, axis=-1, keepdims=True)
    var = jnp.mean(xc * xc, axis=-1, keepdims=True)
    return xc * jax.lax.rsqrt(var + EPS)


def _round(x):
    return x.astype(BF16).astype(F32)


def _kernel(x_hbm, mem_hbm, wq_hbm, wk_hbm, wv_hbm, wo_hbm, wr_hbm, wi_hbm,
            fd_hbm, id_hbm, fs_hbm, is_hbm, o_hbm,
            xb, memb, stage, w, wo, wrb, wib, fd, idm, fs, ism,
            x, h, u, filt, sems, *, S, D, H, Dh, M, seg):
    L = M + seg
    n_seg = S // seg
    nb = S // RADIX
    nc = u.shape[0] // 2
    P = nc * LANES
    Df = wrb.shape[0]
    scale = Dh ** -0.5

    def get(r, c0, n):
        return jnp.concatenate([u[c0 + c, r, :] for c in range(n)], axis=1)

    def put(r, c0, val):
        for c in range(val.shape[1] // LANES):
            u[c0 + c, r, :] = val[:, c * LANES:(c + 1) * LANES]

    started = []

    def fetch(src, dst):
        cp = pltpu.make_async_copy(src, dst, sems.at[len(started)])
        cp.start()
        started.append(cp)
        return cp

    hb = 16
    n_hb = H // hb
    cp_x = fetch(x_hbm, xb)
    cp_filt = [fetch(wr_hbm, wrb), fetch(wi_hbm, wib)]
    cp_w = {}
    for t, src in enumerate((wq_hbm, wk_hbm, wv_hbm)):
        for g in range(n_hb):
            for par in range(2):
                cp_w[t, g, par] = fetch(
                    src.bitcast(jnp.uint32).at[
                        :, pl.ds((par * H + g * hb) // 2, hb // 2), :],
                    stage.at[(t * n_hb + g) * 2 + par].reshape(
                        D // 2, hb // 2, Dh))
    late = [fetch(mem_hbm, memb)]
    late += [fetch(wo_hbm.bitcast(jnp.uint32).at[:, pl.ds(c * LANES, LANES)],
                   wo.at[c])
             for c in range(D // LANES)]
    late += [fetch(fd_hbm, fd), fetch(fs_hbm, fs), fetch(is_hbm, ism),
             fetch(id_hbm, idm)]

    cp_x.wait()

    @pl.loop(0, S // LANES)
    def _(i):
        r = pl.ds(pl.multiple_of(i * LANES, LANES), LANES)
        xv = xb[r, :].astype(F32)
        x[r, :] = xv
        h[r, :] = _layernorm(xv)

    for half, (cp, ref) in enumerate(zip(cp_filt, (wrb, wib))):
        cp.wait()

        @pl.loop(0, S // LANES)
        def _(i):
            r = pl.ds(pl.multiple_of(i * LANES, LANES), LANES)
            v = jnp.concatenate(
                [ref[:, r].astype(F32), jnp.zeros((P - Df, LANES), F32)], 0)
            put(r, half * nc, v.T)

    @pl.loop(0, RADIX)
    def _(f1):
        filt[f1] = get(pl.ds(f1, nb, stride=RADIX), 0, 2 * nc)

    for t in range(3):
        for g in range(n_hb):
            cp_w[t, g, 0].wait()
            cp_w[t, g, 1].wait()
            i = (t * n_hb + g) * 2
            for j in range(hb // 2):
                a = stage[i, pl.ds(j, D // 2, stride=hb // 2), :]
                b = stage[i + 1, pl.ds(j, D // 2, stride=hb // 2), :]
                head = t * H + g * hb + 2 * j
                w[head] = (a & jnp.uint32(0xFFFF)) | (b << 16)
                w[head + 1] = (a >> 16) | (b & jnp.uint32(0xFFFF0000))

    for cp in late:
        cp.wait()

    n_grp = H // GROUP
    gw = GROUP * Dh

    def segment(s, mem):
        r = pl.ds(pl.multiple_of(s * seg, seg), seg)
        hs = jnp.concatenate([mem, h[r, :]], axis=0)
        row = jax.lax.broadcasted_iota(jnp.int32, (L, L), 0)
        col = jax.lax.broadcasted_iota(jnp.int32, (L, L), 1)
        mask = (row < M) | (row >= col)

        def project(g):
            q, k, v = [_dot(hs, _unpack(
                [w[t * H + g * GROUP + j] for j in range(GROUP)]))
                for t in range(3)]
            return q, k.astype(BF16), v.astype(BF16)

        def probs(q, k):
            out = []
            for j in range(GROUP):
                c = slice(j * Dh, (j + 1) * Dh)
                sc = jnp.where(mask, _dot_t(q[:, c], k[:, c]) * scale, NEG)
                e = jnp.exp(sc - jnp.max(sc, axis=-1, keepdims=True))
                out.append((e, pltpu.reciprocal(
                    jnp.sum(e, axis=-1, keepdims=True), approx=True)))
            return out

        def attend(ps, v):
            return jnp.concatenate(
                [_dot(e, v[:, j * Dh:(j + 1) * Dh]) * inv
                 for j, (e, inv) in enumerate(ps)], axis=1)

        qkv, ps, os_ = {}, {}, {}
        acc = None
        for t in range(n_grp + 3):
            if t < n_grp:
                qkv[t] = project(t)
            if 0 <= t - 1 < n_grp:
                ps[t - 1] = probs(qkv[t - 1][0], qkv[t - 1][1])
            if 0 <= t - 2 < n_grp:
                os_[t - 2] = attend(ps[t - 2], qkv[t - 2][2])
            if 0 <= t - 3 < n_grp:
                g = t - 3
                y = _dot(os_[g], _unpack(
                    [wo[c, g * gw // 2:(g + 1) * gw // 2, :]
                     for c in range(D // LANES)]))
                acc = y if acc is None else acc + y
        x[r, :] += acc[M:]
        return acc[:M]

    def butterflies(sign):
        @pl.loop(0, nb // 8)
        def _(i):
            for c in range(nc):
                rows = [pl.ds(pl.multiple_of(a * nb + i * 8, 8), 8)
                        for a in range(RADIX)]
                out = _fft([(u[c, r, :], u[nc + c, r, :]) for r in rows], sign)
                for r, (vr, vi) in zip(rows, out):
                    u[c, r, :] = vr
                    u[nc + c, r, :] = vi

    def spectral():
        blk = 256

        @pl.loop(0, S // blk)
        def _(i):
            r = pl.ds(pl.multiple_of(i * blk, blk), blk)
            put(r, 0, _dot(_layernorm(x[r, :]), fd[...]))

        butterflies(-1)

        @pl.loop(0, RADIX)
        def _(f1):
            r = pl.ds(pl.multiple_of(f1 * nb, nb), nb)
            z = jnp.concatenate([get(r, 0, nc), get(r, nc, nc)],
                                axis=0).astype(BF16)
            y = _dot(fs[f1], z)
            yr, yi = y[:nb], y[nb:]
            wr, wi = filt[f1, :, :P], filt[f1, :, P:]
            z = jnp.concatenate([yr * wr - yi * wi, yr * wi + yi * wr],
                                axis=0).astype(BF16)
            y = _dot(ism[f1], z)
            put(r, 0, y[:nb])
            put(r, nc, y[nb:])

        butterflies(1)

        @pl.loop(0, S // blk)
        def _(i):
            r = pl.ds(pl.multiple_of(i * blk, blk), blk)
            y = _dot(get(r, 0, 2 * nc), idm[...])
            xn = x[r, :] + y
            x[r, :] = xn
            h[r, :] = _layernorm(xn)

    @pl.loop(0, 2)
    def _(layer):
        jax.lax.fori_loop(0, n_seg, segment, memb[...].astype(F32))
        spectral()

    xb[...] = x[...].astype(BF16)
    pltpu.sync_copy(xb, o_hbm)


@functools.partial(jax.jit, static_argnames=("A_seg_len",))
def pallas_interleave_layers__memory_aug_recurrent_mem_tr__spectral_gfnet__prompt_kernel(
    A_x, A_mem0, A_Wq, A_Wk, A_Wv, A_Wo, A_seg_len, B_x, B_w_r, B_w_i,
):
    del B_x
    B, S, D = A_x.shape
    _, H, Dh = A_Wq.shape
    M = A_mem0.shape[1]
    assert B == 1 and Dh == LANES and S == RADIX * LANES and D % LANES == 0
    consts = [c.astype(BF16) for c in _dft_constants(S, D)]
    P2 = consts[0].shape[1]
    hb = 16
    n_w = 3 * 2 * (H // hb)
    args = [A_x.reshape(S, D), A_mem0.reshape(M, D),
            A_Wq.reshape(D // 2, 2 * H, Dh), A_Wk.reshape(D // 2, 2 * H, Dh),
            A_Wv.reshape(D // 2, 2 * H, Dh), A_Wo.reshape(H * Dh, D),
            B_w_r.T, B_w_i.T] + consts
    out = pl.pallas_call(
        functools.partial(_kernel, S=S, D=D, H=H, Dh=Dh, M=M, seg=A_seg_len),
        out_shape=jax.ShapeDtypeStruct((S, D), BF16),
        in_specs=[pl.BlockSpec(memory_space=pltpu.HBM)] * len(args),
        out_specs=pl.BlockSpec(memory_space=pltpu.HBM),
        scratch_shapes=[
            pltpu.VMEM((S, D), BF16),
            pltpu.VMEM((M, D), BF16),
            pltpu.VMEM((n_w, D * hb // 4, Dh), jnp.uint32),
            pltpu.VMEM((3 * H, D // 2, Dh), jnp.uint32),
            pltpu.VMEM((D // LANES, H * Dh // 2, LANES), jnp.uint32),
            pltpu.VMEM(B_w_r.shape[::-1], BF16),
            pltpu.VMEM(B_w_i.shape[::-1], BF16),
        ] + [pltpu.VMEM(c.shape, BF16) for c in consts] + [
            pltpu.VMEM((S, D), F32),
            pltpu.VMEM((S, D), F32),
            pltpu.VMEM((P2 // LANES, S, LANES), F32),
            pltpu.VMEM((RADIX, S // RADIX, P2), F32),
            pltpu.SemaphoreType.DMA((8 + D // LANES + n_w,)),
        ],
        compiler_params=pltpu.CompilerParams(vmem_limit_bytes=100 * 2 ** 20),
    )(*args)
    return out.reshape(B, S, D)
```

```python
import functools
import math

import jax
import jax.numpy as jnp
import numpy as np
import jax.experimental.pallas as pl
import jax.experimental.pallas.tpu as pltpu

F32 = jnp.float32
BF16 = jnp.bfloat16
LANES = 128
RADIX = 16
GROUP = 4
UN_D = 1
UN_S = 1
EPS = 1e-5
NEG = -1000000000.0


def _pack(a):
    bits = a.astype(np.float32).astype(BF16).view(np.uint16).astype(np.uint32)
    words = bits[..., 0::2, :] | (bits[..., 1::2, :] << 16)
    words = words.reshape(words.shape[:-1] + (-1, LANES))
    return np.ascontiguousarray(np.swapaxes(words, -2, -3))


def _dft_constants(S, D):
    j = np.arange(LANES)
    b = j[:, None]
    fwd_d, inv_d = [], []
    for k1 in range(3):
        k = np.where(j < 64, k1 + 5 * j, D - (5 - k1) - 5 * (j - 64))
        wgt = np.full((LANES,), 2.0)
        if k1 == 0:
            k = 5 * j
            wgt = np.where(j < 64, 2.0, 0.0)
            wgt[0] = wgt[64] = 1.0
        ang = 2.0 * np.pi * ((b * k) % D) / D
        c, s = np.cos(ang), np.sin(ang)
        s[:, (2 * k) % D == 0] = 0.0
        m = np.block([[c, -s], [s, c]])
        fwd_d.append(m)
        inv_d.append(m.T * np.tile(wgt, 2)[:, None] / D)
    f = np.arange(RADIX)[:, None, None] + RADIX * j[None, :, None]
    ang = 2.0 * np.pi * ((j[None, None, :] * f) % S) / S
    c, s = np.cos(ang), np.sin(ang)
    fwd_s = np.concatenate([np.concatenate([c, s], 2),
                            np.concatenate([-s, c], 2)], 1)
    inv_s = np.swapaxes(fwd_s, 1, 2) / S
    return [_pack(a) for a in (np.stack(fwd_d), np.stack(inv_d), fwd_s, inv_s)]


def _fft(vals, sign):
    n = len(vals)
    if n == 1:
        return vals
    ev, od = _fft(vals[0::2], sign), _fft(vals[1::2], sign)
    lo, hi = [], []
    for j in range(n // 2):
        (er, ei), (pr, pi) = ev[j], od[j]
        if 4 * j == n:
            if sign > 0:
                lo.append((er - pi, ei + pr))
                hi.append((er + pi, ei - pr))
            else:
                lo.append((er + pi, ei - pr))
                hi.append((er - pi, ei + pr))
            continue
        if j > 0:
            c = math.cos(2 * math.pi * j / n)
            s = sign * math.sin(2 * math.pi * j / n)
            if 8 * j == n:
                pr, pi = ((pr - pi) * c, (pr + pi) * c) if sign > 0 else (
                    (pr + pi) * c, (pi - pr) * c)
            elif 8 * j == 3 * n:
                pr, pi = ((pr + pi) * c, (pi - pr) * c) if sign > 0 else (
                    (pr - pi) * c, (pr + pi) * c)
            else:
                pr, pi = pr * c - pi * s, pr * s + pi * c
        lo.append((er + pr, ei + pi))
        hi.append((er - pr, ei - pi))
    return lo + hi


def _dot(a, b):
    return jax.lax.dot_general(a, b, (((1,), (0,)), ((), ())),
                               preferred_element_type=F32)


def _dot_t(a, b):
    return jax.lax.dot_general(a, b, (((1,), (1,)), ((), ())),
                               preferred_element_type=F32)


def _unpack(tiles):
    return pltpu.bitcast(jnp.concatenate(tiles, axis=1), BF16)


def _layernorm(x):
    xc = x - jnp.mean(x, axis=-1, keepdims=True)
    var = jnp.mean(xc * xc, axis=-1, keepdims=True)
    return xc * jax.lax.rsqrt(var + EPS)


def _iota(shape, axis):
    return jax.lax.broadcasted_iota(jnp.int32, shape, axis)


def _kernel(x_hbm, mem_hbm, wq_hbm, wk_hbm, wv_hbm, wo_hbm, wr_hbm, wi_hbm,
            fd_hbm, id_hbm, fs_hbm, is_hbm, o_hbm,
            x, memb, stage, w, wo, wrb, wib, fd, idm, fs, ism,
            h, ub, u, filt, sems, out_sem, *, S, D, H, Dh, M, seg):
    L = M + seg
    n_seg = S // seg
    nb = LANES
    nc = 3
    P = nc * LANES
    Df = wrb.shape[0]
    scale = Dh ** -0.5

    started = []

    def fetch(src, dst):
        cp = pltpu.make_async_copy(src, dst, sems.at[len(started)])
        cp.start()
        started.append(cp)
        return cp

    hb = 16
    n_hb = H // hb
    cp_filt = [fetch(wr_hbm, wrb), fetch(wi_hbm, wib)]
    cp_w = {}
    for t, src in enumerate((wq_hbm, wk_hbm, wv_hbm)):
        for g in range(n_hb):
            for par in range(2):
                cp_w[t, g, par] = fetch(
                    src.bitcast(jnp.uint32).at[
                        :, pl.ds((par * H + g * hb) // 2, hb // 2), :],
                    stage.at[(t * n_hb + g) * 2 + par].reshape(
                        D // 2, hb // 2, Dh))
    first = [fetch(mem_hbm, memb), fetch(x_hbm.at[0], x.at[0])]
    first += [fetch(wo_hbm.bitcast(jnp.uint32).at[:, pl.ds(c * LANES, LANES)],
                    wo.at[c])
              for c in range(D // LANES)]
    rest = pl.ds(1, RADIX - 1)
    cp_x = fetch(x_hbm.at[rest], x.at[rest])
    cp_dft = [fetch(fd_hbm, fd), fetch(fs_hbm, fs), fetch(is_hbm, ism),
              fetch(id_hbm, idm)]

    j = _iota((P, P), 1) % LANES
    k1 = _iota((P, P), 1) // LANES
    src_bin = jnp.where((j < 64) | (k1 == 0), k1 + 5 * j,
                        (5 - k1) + 5 * (j - 64))
    select = jnp.where(_iota((P, P), 0) == src_bin, 1.0, 0.0).astype(BF16)
    for half, (cp, ref) in enumerate(zip(cp_filt, (wrb, wib))):
        cp.wait()

        @pl.loop(0, S // LANES)
        def _(i):
            r = pl.ds(pl.multiple_of(i * LANES, LANES), LANES)
            v = jnp.concatenate(
                [ref[:, r].astype(F32), jnp.zeros((P - Df, LANES), F32)], 0)
            v = _dot(v.T, select)
            for c in range(nc):
                u[half * nc + c, r, :] = v[:, c * LANES:(c + 1) * LANES]

    @pl.loop(0, RADIX)
    def _(f1):
        pos = _iota((nb, nb), 0) + _iota((nb, nb), 1) + jnp.minimum(f1, 1)
        flip = jnp.where(pos % nb == 0, 1.0, 0.0)
        direct = _iota((nb, LANES), 1) < 64
        for c in range(2 * nc):
            v = u[c, pl.ds(f1, nb, stride=RADIX), :]
            if c % nc:
                m = u[c, pl.ds((RADIX - f1) % RADIX, nb, stride=RADIX), :]
                m = _dot(flip, m.astype(BF16))
                v = jnp.where(direct, v, m if c < nc else -m)
            filt[f1, :, c * LANES:(c + 1) * LANES] = v

    for t in range(3):
        for g in range(n_hb):
            cp_w[t, g, 0].wait()
            cp_w[t, g, 1].wait()
            i = (t * n_hb + g) * 2

            @pl.loop(0, hb // 2)
            def _(j):
                a = stage[i, pl.ds(j, D // 2, stride=hb // 2), :]
                b = stage[i + 1, pl.ds(j, D // 2, stride=hb // 2), :]
                head = t * H + g * hb + 2 * j
                w[head] = (a & jnp.uint32(0xFFFF)) | (b << 16)
                w[head + 1] = (a >> 16) | (b & jnp.uint32(0xFFFF0000))

    for cp in first:
        cp.wait()

    n_grp = H // GROUP
    gw = GROUP * Dh

    def rows_of(s):
        per = nb // seg
        return x.at[s // per, pl.ds(pl.multiple_of(s % per * seg, seg), seg)]

    def segment(layer, s, mem):
        @pl.when((layer == 0) & (s == 1))
        def _():
            cp_x.wait()

        hs = jnp.concatenate([mem, h[s % 2]], axis=0)
        nxt = rows_of(jnp.minimum(s + 1, n_seg - 1))
        h[(s + 1) % 2] = _layernorm(nxt[...].astype(F32))
        row, col = _iota((L, L), 0), _iota((L, L), 1)
        mask = (row < M) | (row >= col)

        def project(g):
            q, k, v = [_dot(hs, _unpack(
                [w[t * H + g * GROUP + j] for j in range(GROUP)]))
                for t in range(3)]
            return q, k.astype(BF16), v.astype(BF16)

        def probs(q, k):
            out = []
            for j in range(GROUP):
                c = slice(j * Dh, (j + 1) * Dh)
                sc = jnp.where(mask, _dot_t(q[:, c], k[:, c]) * scale, NEG)
                e = jnp.exp(sc - jnp.max(sc, axis=-1, keepdims=True))
                out.append((e, pltpu.reciprocal(
                    jnp.sum(e, axis=-1, keepdims=True), approx=True)))
            return out

        def attend(ps, v):
            return jnp.concatenate(
                [_dot(e, v[:, j * Dh:(j + 1) * Dh]) * inv
                 for j, (e, inv) in enumerate(ps)], axis=1)

        qkv, ps, os_ = {}, {}, {}
        acc = None
        for t in range(n_grp + 3):
            if t < n_grp:
                qkv[t] = project(t)
            if 0 <= t - 1 < n_grp:
                ps[t - 1] = probs(qkv[t - 1][0], qkv[t - 1][1])
            if 0 <= t - 2 < n_grp:
                os_[t - 2] = attend(ps[t - 2], qkv[t - 2][2])
            if 0 <= t - 3 < n_grp:
                g = t - 3
                y = _dot(os_[g], _unpack(
                    [wo[c, g * gw // 2:(g + 1) * gw // 2, :]
                     for c in range(D // LANES)]))
                acc = y if acc is None else acc + y
        cur = rows_of(s)
        cur[...] = (cur[...].astype(F32) + acc[M:]).astype(BF16)
        return acc[:M]

    c1, c2 = math.cos(0.4 * math.pi), math.cos(0.8 * math.pi)
    s1, s2 = math.sin(0.4 * math.pi), math.sin(0.8 * math.pi)
    ch = 16

    def tiles(v):
        return [v[:, c:c + LANES] for c in range(0, v.shape[1], LANES)]

    def spectral(layer):
        @pl.loop(0, nb // ch, unroll=UN_D)
        def _(i):
            r = pl.ds(pl.multiple_of(i * ch, ch), ch)
            t = tiles(_layernorm(
                x[:, r, :].astype(F32).reshape(RADIX * ch, D)))
            a1, a2, d1, d2 = t[1] + t[4], t[2] + t[3], t[4] - t[1], t[3] - t[2]
            parts = [[t[0] + a1 + a2],
                     [t[0] + c1 * a1 + c2 * a2, s1 * d1 + s2 * d2],
                     [t[0] + c2 * a1 + c1 * a2, s2 * d1 - s1 * d2]]
            o = pl.multiple_of(i * (ch // 2), ch // 2)
            for c, p in enumerate(parts):
                k = len(p) * LANES // 2
                re, im = tiles(_dot(jnp.concatenate(p, axis=1),
                                    _unpack([fd[c, 0, :k], fd[c, 1, :k]])))
                out = _fft([(re[a * ch:(a + 1) * ch], im[a * ch:(a + 1) * ch])
                            for a in range(RADIX)], -1)
                for f1, v in enumerate(out):
                    for half in range(2):
                        ub[f1, c, pl.ds(o + half * nb // 2, ch // 2), :] = (
                            pltpu.bitcast(v[half].astype(BF16), jnp.uint32))

        @pl.loop(0, RADIX, unroll=UN_S)
        def _(f1):
            y = _dot(_unpack([fs[f1, 0], fs[f1, 1]]),
                     _unpack([ub[f1, c] for c in range(nc)]))
            yr, yi = y[:nb], y[nb:]
            wr, wi = filt[f1, :, :P], filt[f1, :, P:]
            z = jnp.concatenate([yr * wr - yi * wi, yr * wi + yi * wr],
                                axis=0).astype(BF16)
            y = _dot(_unpack([ism[f1, 0], ism[f1, 1]]), z)
            r = pl.ds(pl.multiple_of(f1 * nb, nb), nb)
            for c, v in enumerate(tiles(y[:nb]) + tiles(y[nb:])):
                u[c, r, :] = v

        @pl.loop(0, nb // ch, unroll=UN_D)
        def _(i):
            rows = [pl.ds(pl.multiple_of(f1 * nb + i * ch, ch), ch)
                    for f1 in range(RADIX)]
            g = []
            for c in range(nc):
                out = _fft([(u[c, r, :], u[nc + c, r, :]) for r in rows], 1)
                z = jnp.concatenate(
                    [jnp.concatenate(v, axis=1) for v in out], axis=0)
                g += tiles(_dot(z, _unpack(
                    [idm[c, n] for n in range(2 if c else 1)])))
            g0, g1r, g1i, g2r, g2i = g
            a1, a2 = g0 + c1 * g1r + c2 * g2r, g0 + c2 * g1r + c1 * g2r
            b1, b2 = s1 * g1i + s2 * g2i, s2 * g1i - s1 * g2i
            y = jnp.concatenate(
                [g0 + g1r + g2r, a1 - b1, a2 - b2, a2 + b2, a1 + b1], axis=1)
            r = pl.ds(pl.multiple_of(i * ch, ch), ch)
            x[:, r, :] = (x[:, r, :].astype(F32)
                          + y.reshape(RADIX, ch, D)).astype(BF16)

            @pl.when(layer == 1)
            def _():
                pltpu.make_async_copy(x.at[:, r, :], o_hbm.at[:, r, :],
                                      out_sem).start()

    @pl.loop(0, 2)
    def _(layer):
        h[0] = _layernorm(x[0, :seg, :].astype(F32))
        jax.lax.fori_loop(0, n_seg, functools.partial(segment, layer),
                          memb[...].astype(F32))

        @pl.when(layer == 0)
        def _():
            for cp in cp_dft:
                cp.wait()

        spectral(layer)

    pltpu.make_async_copy(x, o_hbm, out_sem).wait()


@functools.partial(jax.jit, static_argnames=("A_seg_len",))
def pallas_interleave_layers__memory_aug_recurrent_mem_tr__spectral_gfnet__prompt_kernel(
    A_x, A_mem0, A_Wq, A_Wk, A_Wv, A_Wo, A_seg_len, B_x, B_w_r, B_w_i,
):
    del B_x
    B, S, D = A_x.shape
    _, H, Dh = A_Wq.shape
    M = A_mem0.shape[1]
    assert B == 1 and Dh == LANES and S == RADIX * LANES and D == 5 * LANES
    consts = _dft_constants(S, D)
    n_w = 3 * 2 * (H // 16)
    args = [A_x.reshape(RADIX, LANES, D), A_mem0.reshape(M, D),
            A_Wq.reshape(D // 2, 2 * H, Dh), A_Wk.reshape(D // 2, 2 * H, Dh),
            A_Wv.reshape(D // 2, 2 * H, Dh), A_Wo.reshape(H * Dh, D),
            B_w_r.T, B_w_i.T] + consts
    u32 = jnp.uint32
    out = pl.pallas_call(
        functools.partial(_kernel, S=S, D=D, H=H, Dh=Dh, M=M, seg=A_seg_len),
        out_shape=jax.ShapeDtypeStruct((RADIX, LANES, D), BF16),
        in_specs=[pl.BlockSpec(memory_space=pltpu.HBM)] * len(args),
        out_specs=pl.BlockSpec(memory_space=pltpu.HBM),
        scratch_shapes=[
            pltpu.VMEM((RADIX, LANES, D), BF16),
            pltpu.VMEM((M, D), BF16),
            pltpu.VMEM((n_w, D * 4, Dh), u32),
            pltpu.VMEM((3 * H, D // 2, Dh), u32),
            pltpu.VMEM((D // LANES, H * Dh // 2, LANES), u32),
            pltpu.VMEM(B_w_r.shape[::-1], BF16),
            pltpu.VMEM(B_w_i.shape[::-1], BF16),
        ] + [pltpu.VMEM(c.shape, u32) for c in consts] + [
            pltpu.VMEM((2, A_seg_len, D), F32),
            pltpu.VMEM((RADIX, 3, LANES, LANES), u32),
            pltpu.VMEM((6, S, LANES), F32),
            pltpu.VMEM((RADIX, LANES, 6 * LANES), F32),
            pltpu.SemaphoreType.DMA((9 + D // LANES + n_w,)),
            pltpu.SemaphoreType.DMA(()),
        ],
        compiler_params=pltpu.CompilerParams(vmem_limit_bytes=100 * 2 ** 20),
    )(*args)
    return out.reshape(B, S, D)
```

```python
import functools
import math

import jax
import jax.numpy as jnp
import numpy as np
import jax.experimental.pallas as pl
import jax.experimental.pallas.tpu as pltpu

F32 = jnp.float32
BF16 = jnp.bfloat16
LANES = 128
RADIX = 32
GROUP = 4
UN_D = True
LAG = 2
PRE = 10
UN_A = 2
EPS = 1e-5
NEG = -1000000000.0


def _pack(a):
    bits = a.astype(np.float32).astype(BF16).view(np.uint16).astype(np.uint32)
    words = bits[..., 0::2, :] | (bits[..., 1::2, :] << 16)
    words = words.reshape(words.shape[:-1] + (-1, LANES))
    return np.ascontiguousarray(np.swapaxes(words, -2, -3))


def _dft_constants(S, D):
    j = np.arange(LANES)
    b = j[:, None]
    fwd_d, inv_d = [], []
    for k1 in range(3):
        k = np.where(j < 64, k1 + 5 * j, D - (5 - k1) - 5 * (j - 64))
        wgt = np.full((LANES,), 2.0)
        if k1 == 0:
            k = 5 * j
            wgt = np.where(j < 64, 2.0, 0.0)
            wgt[0] = wgt[64] = 1.0
        ang = 2.0 * np.pi * ((b * k) % D) / D
        c, s = np.cos(ang), np.sin(ang)
        s[:, (2 * k) % D == 0] = 0.0
        m = np.block([[c, -s], [s, c]])
        fwd_d.append(m)
        inv_d.append(m.T * np.tile(wgt, 2)[:, None] / D)
    j = np.arange(S // RADIX)
    f = np.arange(RADIX)[:, None, None] + RADIX * j[None, :, None]
    ang = 2.0 * np.pi * ((j[None, None, :] * f) % S) / S
    c, s = np.cos(ang), np.sin(ang)
    fwd_s = np.concatenate([np.concatenate([c, s], 2),
                            np.concatenate([-s, c], 2)], 1)
    inv_s = np.swapaxes(fwd_s, 1, 2) / S
    return [_pack(a) for a in (np.stack(fwd_d), np.stack(inv_d), fwd_s, inv_s)]


def _fft(vals, sign):
    n = len(vals)
    if n == 1:
        return vals
    ev, od = _fft(vals[0::2], sign), _fft(vals[1::2], sign)
    lo, hi = [], []
    for j in range(n // 2):
        (er, ei), (pr, pi) = ev[j], od[j]
        if 4 * j == n:
            if sign > 0:
                lo.append((er - pi, ei + pr))
                hi.append((er + pi, ei - pr))
            else:
                lo.append((er + pi, ei - pr))
                hi.append((er - pi, ei + pr))
            continue
        if j > 0:
            c = math.cos(2 * math.pi * j / n)
            s = sign * math.sin(2 * math.pi * j / n)
            if 8 * j == n:
                pr, pi = ((pr - pi) * c, (pr + pi) * c) if sign > 0 else (
                    (pr + pi) * c, (pi - pr) * c)
            elif 8 * j == 3 * n:
                pr, pi = ((pr + pi) * c, (pi - pr) * c) if sign > 0 else (
                    (pr - pi) * c, (pr + pi) * c)
            else:
                pr, pi = pr * c - pi * s, pr * s + pi * c
        lo.append((er + pr, ei + pi))
        hi.append((er - pr, ei - pi))
    return lo + hi


def _dot(a, b):
    return jax.lax.dot_general(a, b, (((1,), (0,)), ((), ())),
                               preferred_element_type=F32)


def _dot_t(a, b):
    return jax.lax.dot_general(a, b, (((1,), (1,)), ((), ())),
                               preferred_element_type=F32)


def _unpack(tiles):
    return pltpu.bitcast(jnp.concatenate(tiles, axis=1), BF16)


def _layernorm(x):
    xc = x - jnp.mean(x, axis=-1, keepdims=True)
    var = jnp.mean(xc * xc, axis=-1, keepdims=True)
    return xc * jax.lax.rsqrt(var + EPS)


def _iota(shape, axis):
    return jax.lax.broadcasted_iota(jnp.int32, shape, axis)


def _kernel(x_hbm, mem_hbm, wq_hbm, wk_hbm, wv_hbm, wo_hbm, wr_hbm, wi_hbm,
            fd_hbm, id_hbm, fs_hbm, is_hbm, o_hbm,
            x, memb, stage, w, wo, wrb, wib, fd, idm, fs, ism,
            xt, ht, pre, h, fx, ub, u, filt, sems, out_sem, *, S, D, H, Dh, M, seg):
    L = M + seg
    n_seg = S // seg
    nb = S // RADIX
    nc = 3
    P = nc * LANES
    Df = wrb.shape[0]
    scale = Dh ** -0.5

    started = []

    def fetch(src, dst):
        cp = pltpu.make_async_copy(src, dst, sems.at[len(started)])
        cp.start()
        started.append(cp)
        return cp

    pitch = stage.shape[1] // (D // 2)
    per = nb // seg
    cp_filt = [fetch(wr_hbm, wrb), fetch(wi_hbm, wib)]
    cp_tail = [fetch(x_hbm.at[:, pl.ds((n + 1) * seg - 8, 8)], xt.at[n])
               for n in range(per)]
    cp_w = [fetch(src.bitcast(jnp.uint32).at[:, pl.ds(par * H // 2, H // 2)],
                  stage.at[2 * t + par].reshape(D // 2, pitch, Dh)
                  .at[:, pl.ds(0, H // 2)])
            for t, src in enumerate((wq_hbm, wk_hbm, wv_hbm))
            for par in range(2)]
    n0 = pl.cdiv((UN_A + 1) * seg, nb)
    first = [fetch(mem_hbm, memb), fetch(x_hbm.at[:n0], x.at[:n0])]
    first += [fetch(wo_hbm.bitcast(jnp.uint32).at[:, pl.ds(c * LANES, LANES)],
                    wo.at[c])
              for c in range(D // LANES)]

    gap = RADIX + 8
    n_tmp = 4
    for half, (cp, ref) in enumerate(zip(cp_filt, (wrb, wib))):
        cp.wait()

        @pl.loop(0, S // LANES // n_tmp)
        def _(i):
            for n in range(n_tmp):
                r = pl.ds(pl.multiple_of((i * n_tmp + n) * LANES, LANES),
                          LANES)
                pre[n, :P, :] = jnp.concatenate(
                    [ref[:, r].astype(F32), jnp.zeros((P - Df, LANES), F32)],
                    0)
            for n in range(n_tmp):
                def bins(k0, cnt):
                    return pre[n, pl.ds(k0, cnt, stride=5), :]
                lines = [[bins(0, 72), jnp.zeros((56, LANES), F32)],
                         [bins(1, 64), bins(4, 64)],
                         [bins(2, 64), bins(3, 64)]]
                for c, pair in enumerate(lines):
                    v = jnp.concatenate(pair, axis=0).T
                    for m in range(LANES // RADIX):
                        o = ((i * n_tmp + n) * (LANES // RADIX) + m) * gap
                        u[half * nc + c,
                          pl.ds(pl.multiple_of(o, 8), RADIX), :] = (
                              v[m * RADIX:(m + 1) * RADIX])

    @pl.loop(0, RADIX, unroll=4)
    def _(f1):
        pos = _iota((nb, nb), 0) + _iota((nb, nb), 1) + jnp.minimum(f1, 1)
        flip = jnp.where((pos == 0) | (pos == nb), 1.0, 0.0)
        direct = _iota((nb, LANES), 1) < 64
        for c in range(2 * nc):
            v = u[c, pl.ds(f1, nb, stride=gap), :]
            if c % nc:
                m = u[c, pl.ds((RADIX - f1) % RADIX, nb, stride=gap), :]
                m = _dot(flip, m.astype(BF16))
                v = jnp.where(direct, v, m if c < nc else -m)
            filt[f1, :, c * LANES:(c + 1) * LANES] = v

    for cp in cp_tail:
        cp.wait()
    ht[...] = _layernorm(xt[...].astype(F32).reshape(n_seg * 8, D))

    n_grp = H // GROUP

    def regroup(t, g):
        out = []
        for n in range(GROUP // 2):
            j = pl.ds(g * (GROUP // 2) + n, D // 2, stride=pitch)
            a, b = stage[2 * t, j, :], stage[2 * t + 1, j, :]
            out += [(a & jnp.uint32(0xFFFF)) | (b << 16),
                    (a >> 16) | (b & jnp.uint32(0xFFFF0000))]
        for n, v in enumerate(out):
            w[t * H + g * GROUP + n] = v
        return out

    for t in range(3):
        cp_w[2 * t].wait()
        cp_w[2 * t + 1].wait()
        n_pre = min(max(PRE - t * n_grp, 0), n_grp)
        if n_pre:
            @pl.loop(0, n_pre, unroll=2)
            def _(g):
                y = _dot(ht[...], _unpack(regroup(t, g)))
                for n in range(GROUP):
                    pre[t * H + g * GROUP + n] = y[:, n * Dh:(n + 1) * Dh]

        if n_pre < n_grp:
            pl.loop(n_pre, n_grp)(lambda g: regroup(t, g) and None)

    for cp in first:
        cp.wait()
    rest = pl.ds(n0, RADIX - n0)
    cp_x = fetch(x_hbm.at[rest], x.at[rest])
    cp_dft = [fetch(fd_hbm, fd), fetch(fs_hbm, fs), fetch(is_hbm, ism),
              fetch(id_hbm, idm)]

    gw = GROUP * Dh

    c1, c2 = math.cos(0.4 * math.pi), math.cos(0.8 * math.pi)
    s1, s2 = math.sin(0.4 * math.pi), math.sin(0.8 * math.pi)
    ch = 16

    def tiles(v):
        return [v[:, c:c + LANES] for c in range(0, v.shape[1], LANES)]

    def fold(s):
        t = tiles(_layernorm(rows_of(s)[...].astype(F32)))
        a1, a2, d1, d2 = t[1] + t[4], t[2] + t[3], t[4] - t[1], t[3] - t[2]
        rows_of(s, fx)[...] = jnp.concatenate(
            [t[0] + a1 + a2,
             t[0] + c1 * a1 + c2 * a2, s1 * d1 + s2 * d2,
             t[0] + c2 * a1 + c1 * a2, s2 * d1 - s1 * d2], axis=1)

    def rows_of(s, ref=x):
        return ref.at[s // per, pl.ds(pl.multiple_of(s % per * seg, seg), seg)]

    def segments(layer, i, mem):
        if layer == 0:
            pl.when(i == 1)(cp_x.wait)
        for n in range(UN_A):
            mem = segment(layer, i * UN_A + n, n % 2, mem)
        return mem

    def segment(layer, s, slot, mem):
        hs = jnp.concatenate([mem, h[slot]], axis=0)
        nxt = rows_of(jnp.minimum(s + 1, n_seg - 1))
        h[1 - slot] = _layernorm(nxt[...].astype(F32))
        fold(jnp.maximum(s - 1, 0))
        row, col = _iota((L, L), 0), _iota((L, L), 1)
        mask = (row < M) | (row >= col)

        tail = pl.ds(pl.multiple_of((s % per * RADIX + s // per) * 8, 8), 8)

        def linear(g):
            heads = range(g * GROUP, (g + 1) * GROUP)
            wg = _unpack([w[j] for j in heads])
            if layer > 0 or g >= PRE:
                return _dot(hs, wg)
            done = jnp.concatenate([pre[j, tail, :] for j in heads], axis=1)
            return jnp.concatenate([_dot(hs[:L - 8], wg), done], axis=0)

        def project(g):
            q, k, v = [linear(t * n_grp + g) for t in range(3)]
            return q, k.astype(BF16), v.astype(BF16)

        def probs(q, k):
            out = []
            for j in range(GROUP):
                c = slice(j * Dh, (j + 1) * Dh)
                sc = jnp.where(mask, _dot_t(q[:, c], k[:, c]) * scale, NEG)
                e = jnp.exp(sc - jnp.max(sc, axis=-1, keepdims=True))
                out.append((e, pltpu.reciprocal(
                    jnp.sum(e, axis=-1, keepdims=True), approx=True)))
            return out

        def attend(ps, v):
            return jnp.concatenate(
                [_dot(e, v[:, j * Dh:(j + 1) * Dh]) * inv
                 for j, (e, inv) in enumerate(ps)], axis=1)

        qkv, ps, os_ = {}, {}, {}
        acc = None
        for t in range(n_grp + 3):
            if t < n_grp:
                qkv[t] = project(t)
            if 0 <= t - 1 < n_grp:
                ps[t - 1] = probs(qkv[t - 1][0], qkv[t - 1][1])
            if 0 <= t - 2 < n_grp:
                os_[t - 2] = attend(ps[t - 2], qkv[t - 2][2])
            if 0 <= t - 3 < n_grp:
                g = t - 3
                y = _dot(os_[g], _unpack(
                    [wo[c, g * gw // 2:(g + 1) * gw // 2, :]
                     for c in range(D // LANES)]))
                acc = y if acc is None else acc + y
        cur = rows_of(s)
        cur[...] = (cur[...].astype(F32) + acc[M:]).astype(BF16)
        return acc[:M]

    def spectral(layer):
        fold(n_seg - 1)

        @pl.loop(0, nb // ch, unroll=UN_D)
        def _(i):
            t = tiles(jnp.concatenate(
                [fx[:, pl.ds(i * ch + o, 8), :].reshape(RADIX * 8, D)
                 for o in range(0, ch, 8)], axis=0))
            o = pl.multiple_of(i * (ch // 2), ch // 2)
            for c, p in enumerate([t[:1], t[1:3], t[3:]]):
                k = len(p) * LANES // 2
                re, im = tiles(_dot(jnp.concatenate(p, axis=1),
                                    _unpack([fd[c, 0, :k], fd[c, 1, :k]])))
                out = [_fft([(re[r:r + 8], im[r:r + 8]) for r in
                             range(n * RADIX * 8, (n + 1) * RADIX * 8, 8)], -1)
                       for n in range(ch // 8)]
                for f1 in range(RADIX):
                    for half in range(2):
                        v = jnp.concatenate([q[f1][half] for q in out], 0)
                        ub[f1, c, pl.ds(o + half * nb // 2, ch // 2), :] = (
                            pltpu.bitcast(v.astype(BF16), jnp.uint32))

        zs = {}
        for t in range(RADIX + LAG):
            if t < RADIX:
                y = _dot(_unpack([fs[t, n] for n in range(fs.shape[1])]),
                         _unpack([ub[t, c] for c in range(nc)]))
                yr, yi = y[:nb], y[nb:]
                wr, wi = filt[t, :, :P], filt[t, :, P:]
                zs[t] = jnp.concatenate(
                    [yr * wr - yi * wi, yr * wi + yi * wr], 0).astype(BF16)
            if t >= LAG:
                f1 = t - LAG
                y = _dot(_unpack([ism[f1, n] for n in range(fs.shape[1])]),
                         zs.pop(f1))
                for c, v in enumerate(tiles(y[:nb]) + tiles(y[nb:])):
                    u[c, f1 * nb:(f1 + 1) * nb, :] = v

        @pl.loop(0, nb // ch, unroll=UN_D)
        def _(i):
            g = []
            for c in range(nc):
                parts = []
                for o in range(0, ch, 8):
                    rows = [pl.ds(f1 * nb + i * ch + o, 8)
                            for f1 in range(RADIX)]
                    out = _fft([(u[c, r, :], u[nc + c, r, :]) for r in rows],
                               1)
                    parts += [jnp.concatenate(v, axis=1) for v in out]
                g += tiles(_dot(jnp.concatenate(parts, axis=0), _unpack(
                    [idm[c, n] for n in range(2 if c else 1)])))
            g0, g1r, g1i, g2r, g2i = g
            a1, a2 = g0 + c1 * g1r + c2 * g2r, g0 + c2 * g1r + c1 * g2r
            b1, b2 = s1 * g1i + s2 * g2i, s2 * g1i - s1 * g2i
            y = jnp.concatenate(
                [g0 + g1r + g2r, a1 - b1, a2 - b2, a2 + b2, a1 + b1], axis=1)
            y = y.reshape(ch // 8, RADIX, 8, D)
            y = jnp.concatenate([y[n] for n in range(ch // 8)], axis=1)
            r = pl.ds(pl.multiple_of(i * ch, ch), ch)
            x[:, r, :] = (x[:, r, :].astype(F32) + y).astype(BF16)

            @pl.when(layer == 1)
            def _():
                pltpu.make_async_copy(x.at[:, r, :], o_hbm.at[:, r, :],
                                      out_sem).start()

    @pl.loop(0, 2)
    def _(layer):
        h[0] = _layernorm(x[0, :seg, :].astype(F32))
        for n in range(2):
            @pl.when(layer == n)
            def _():
                jax.lax.fori_loop(0, n_seg // UN_A,
                                  functools.partial(segments, n),
                                  memb[...].astype(F32))
                if n == 0:
                    for cp in cp_dft:
                        cp.wait()

        spectral(layer)

    pltpu.make_async_copy(x, o_hbm, out_sem).wait()


@functools.partial(jax.jit, static_argnames=("A_seg_len",))
def pallas_interleave_layers__memory_aug_recurrent_mem_tr__spectral_gfnet__prompt_kernel(
    A_x, A_mem0, A_Wq, A_Wk, A_Wv, A_Wo, A_seg_len, B_x, B_w_r, B_w_i,
):
    del B_x
    B, S, D = A_x.shape
    _, H, Dh = A_Wq.shape
    M = A_mem0.shape[1]
    assert B == 1 and Dh == LANES and D == 5 * LANES
    consts = _dft_constants(S, D)
    n_w = 6
    n_seg = S // A_seg_len
    per = n_seg // RADIX
    args = [A_x.reshape(RADIX, S // RADIX, D), A_mem0.reshape(M, D),
            A_Wq.reshape(D // 2, 2 * H, Dh), A_Wk.reshape(D // 2, 2 * H, Dh),
            A_Wv.reshape(D // 2, 2 * H, Dh), A_Wo.reshape(H * Dh, D),
            B_w_r.T, B_w_i.T] + consts
    u32 = jnp.uint32
    out = pl.pallas_call(
        functools.partial(_kernel, S=S, D=D, H=H, Dh=Dh, M=M, seg=A_seg_len),
        out_shape=jax.ShapeDtypeStruct((RADIX, S // RADIX, D), BF16),
        in_specs=[pl.BlockSpec(memory_space=pltpu.HBM)] * len(args),
        out_specs=pl.BlockSpec(memory_space=pltpu.HBM),
        scratch_shapes=[
            pltpu.VMEM((RADIX, S // RADIX, D), BF16),
            pltpu.VMEM((M, D), BF16),
            pltpu.VMEM((n_w, D // 2 * 24, Dh), u32),
            pltpu.VMEM((3 * H, D // 2, Dh), u32),
            pltpu.VMEM((D // LANES, H * Dh // 2, LANES), u32),
            pltpu.VMEM(B_w_r.shape[::-1], BF16),
            pltpu.VMEM(B_w_i.shape[::-1], BF16),
        ] + [pltpu.VMEM(c.shape, u32) for c in consts] + [
            pltpu.VMEM((per, RADIX, 8, D), BF16),
            pltpu.VMEM((n_seg * 8, D), F32),
            pltpu.VMEM((PRE * GROUP, n_seg * 8, Dh), F32),
            pltpu.VMEM((2, A_seg_len, D), F32),
            pltpu.VMEM((RADIX, S // RADIX, D), F32),
            pltpu.VMEM((RADIX, 3, S // RADIX, LANES), u32),
            pltpu.VMEM((6, S // RADIX * (RADIX + 8), LANES), F32),
            pltpu.VMEM((RADIX, S // RADIX, 6 * LANES), F32),
            pltpu.SemaphoreType.DMA((9 + D // LANES + n_w + per,)),
            pltpu.SemaphoreType.DMA(()),
        ],
        compiler_params=pltpu.CompilerParams(vmem_limit_bytes=110 * 2 ** 20),
    )(*args)
    return out.reshape(B, S, D)
```

```python
import functools
import math

import jax
import jax.numpy as jnp
import numpy as np
import jax.experimental.pallas as pl
import jax.experimental.pallas.tpu as pltpu

F32 = jnp.float32
BF16 = jnp.bfloat16
LANES = 128
RADIX = 32
GROUP = 4
UN_D = True
LAG = 2
SPLIT = 4
PRE = 14
UN_A = 2
EPS = 1e-5
NEG = -1000000000.0


def _pack(a):
    bits = a.astype(np.float32).astype(BF16).view(np.uint16).astype(np.uint32)
    words = bits[..., 0::2, :] | (bits[..., 1::2, :] << 16)
    words = words.reshape(words.shape[:-1] + (-1, LANES))
    return np.ascontiguousarray(np.swapaxes(words, -2, -3))


def _dft_constants(S, D):
    j = np.arange(LANES)
    b = j[:, None]
    fwd_d, inv_d = [], []
    for k1 in range(3):
        k = np.where(j < 64, k1 + 5 * j, D - (5 - k1) - 5 * (j - 64))
        wgt = np.full((LANES,), 2.0)
        if k1 == 0:
            k = 5 * j
            wgt = np.where(j < 64, 2.0, 0.0)
            wgt[0] = wgt[64] = 1.0
        ang = 2.0 * np.pi * ((b * k) % D) / D
        c, s = np.cos(ang), np.sin(ang)
        s[:, (2 * k) % D == 0] = 0.0
        m = np.block([[c, -s], [s, c]])
        fwd_d.append(m)
        inv_d.append(m.T * np.tile(wgt, 2)[:, None] / D)
    j = np.arange(S // RADIX)
    f = np.arange(RADIX)[:, None, None] + RADIX * j[None, :, None]
    ang = 2.0 * np.pi * ((j[None, None, :] * f) % S) / S
    c, s = np.cos(ang), np.sin(ang)
    fwd_s = np.concatenate([np.concatenate([c, s], 2),
                            np.concatenate([-s, c], 2)], 1)
    inv_s = np.swapaxes(fwd_s, 1, 2) / S
    return [_pack(a) for a in (np.stack(fwd_d), np.stack(inv_d), fwd_s, inv_s)]


def _fft(vals, sign):
    n = len(vals)
    if n == 1:
        return vals
    ev, od = _fft(vals[0::2], sign), _fft(vals[1::2], sign)
    lo, hi = [], []
    for j in range(n // 2):
        (er, ei), (pr, pi) = ev[j], od[j]
        if 4 * j == n:
            if sign > 0:
                lo.append((er - pi, ei + pr))
                hi.append((er + pi, ei - pr))
            else:
                lo.append((er + pi, ei - pr))
                hi.append((er - pi, ei + pr))
            continue
        if j > 0:
            c = math.cos(2 * math.pi * j / n)
            s = sign * math.sin(2 * math.pi * j / n)
            if 8 * j == n:
                pr, pi = ((pr - pi) * c, (pr + pi) * c) if sign > 0 else (
                    (pr + pi) * c, (pi - pr) * c)
            elif 8 * j == 3 * n:
                pr, pi = ((pr + pi) * c, (pi - pr) * c) if sign > 0 else (
                    (pr - pi) * c, (pr + pi) * c)
            else:
                pr, pi = pr * c - pi * s, pr * s + pi * c
        lo.append((er + pr, ei + pi))
        hi.append((er - pr, ei - pi))
    return lo + hi


def _dot(a, b):
    return jax.lax.dot_general(a, b, (((1,), (0,)), ((), ())),
                               preferred_element_type=F32)


def _dot_t(a, b):
    return jax.lax.dot_general(a, b, (((1,), (1,)), ((), ())),
                               preferred_element_type=F32)


def _unpack(tiles):
    return pltpu.bitcast(jnp.concatenate(tiles, axis=1), BF16)


def _layernorm(x):
    xc = x - jnp.mean(x, axis=-1, keepdims=True)
    var = jnp.mean(xc * xc, axis=-1, keepdims=True)
    return xc * jax.lax.rsqrt(var + EPS)


def _iota(shape, axis):
    return jax.lax.broadcasted_iota(jnp.int32, shape, axis)


def _kernel(x_hbm, mem_hbm, wq_hbm, wk_hbm, wv_hbm, wo_hbm, wr_hbm, wi_hbm,
            fd_hbm, id_hbm, fs_hbm, is_hbm, o_hbm,
            x, memb, stage_q, stage, w, w1, wo, wrb, wib, fd, idm, fs, ism,
            tmp, xt, ht, pre, h, fx, ub, u, filt, sems, out_sem, *, S, D, H, Dh, M, seg):
    L = M + seg
    n_seg = S // seg
    nb = S // RADIX
    nc = 3
    P = nc * LANES
    Df = wrb.shape[0]
    scale = Dh ** -0.5

    started = []

    def fetch(src, dst):
        cp = pltpu.make_async_copy(src, dst, sems.at[len(started)])
        cp.start()
        started.append(cp)
        return cp

    per = nb // seg

    def fetch_w(src, buf, slot, lo, n):
        pitch = buf.shape[1] // (D // 2)
        return [fetch(
            src.bitcast(jnp.uint32).at[:, pl.ds(par * H // 2 + lo, n)],
            buf.at[2 * slot + par].reshape(D // 2, pitch, Dh)
            .at[:, pl.ds(0, n)]) for par in range(2)]

    cp_tail = [fetch(x_hbm.at[:, pl.ds((n + 1) * seg - 8, 8)], xt.at[n])
               for n in range(per)]
    cp_q = [fetch_w(wq_hbm, stage_q, n, n * H // 4, H // 4) for n in range(2)]
    cp_filt = [fetch(wr_hbm, wrb), fetch(wi_hbm, wib)]
    cp_k = fetch_w(wk_hbm, stage, 0, 0, H // 2)
    cp_v = fetch_w(wv_hbm, stage, 1, 0, H // 2)
    n0 = pl.cdiv((UN_A + 1) * seg, nb)
    first = [fetch(mem_hbm, memb), fetch(x_hbm.at[:n0], x.at[:n0])]
    first += [fetch(wo_hbm.bitcast(jnp.uint32).at[:, pl.ds(c * LANES, LANES)],
                    wo.at[c])
              for c in range(D // LANES)]

    n_part = tmp.shape[0]
    gap = RADIX + 8

    def transpose_filter(i):
        for n in range(n_part):
            blk = i * (n_part // 2) + n // 2
            r = pl.ds(pl.multiple_of(blk * LANES, LANES), LANES)
            tmp[n] = jnp.concatenate(
                [(wrb, wib)[n % 2][:, r].astype(F32),
                 jnp.zeros((P - Df, LANES), F32)], 0)
            yield
            for c in range(nc):
                v = jnp.concatenate(
                    [tmp[n, pl.ds(c, 64 if c else 72, stride=5), :],
                     tmp[n, pl.ds(5 - c, 64, stride=5), :] if c
                     else jnp.zeros((56, LANES), F32)], axis=0).T
                for m in range(LANES // RADIX):
                    o = pl.multiple_of((blk * (LANES // RADIX) + m) * gap, 8)
                    u[n % 2 * nc + c, pl.ds(o, RADIX), :] = (
                        v[m * RADIX:(m + 1) * RADIX])
                yield

    def gather_filter(i):
        for n in range(n_part):
            f1 = i * n_part + n
            pos = _iota((nb, nb), 0) + _iota((nb, nb), 1) + jnp.minimum(f1, 1)
            flip = jnp.where((pos == 0) | (pos == nb), 1.0, 0.0)
            neg = pl.ds((RADIX - f1) % RADIX, nb, stride=gap)
            mixed = [c for c in range(2 * nc) if c % nc]
            m = _dot(flip, jnp.concatenate(
                [u[c, neg, :] for c in mixed], axis=1).astype(BF16))
            yield
            yield
            for c in range(2 * nc):
                v = u[c, pl.ds(f1, nb, stride=gap), :]
                if c % nc:
                    o = mixed.index(c) * LANES
                    mc = m[:, o:o + LANES]
                    v = jnp.where(_iota((nb, LANES), 1) < 64, v,
                                  mc if c < nc else -mc)
                filt[f1, :, c * LANES:(c + 1) * LANES] = v
                if c % 2:
                    yield

    n_grp = H // GROUP
    kt = LANES // 2

    def regroup(pair, is_q, dst, base):
        buf, n, q = ((stage_q, H // 4, pair) if is_q else
                     (stage, H // 2, pair - H // 2))
        pitch = buf.shape[1] // (D // 2)
        for k in range(0, D // 2, kt):
            j = pl.ds(q % n + k * pitch, kt, stride=pitch)
            a, b = [buf[q // n * 2 + par, j, :] for par in range(2)]
            even = (a & jnp.uint32(0xFFFF)) | (b << 16)
            odd = (a >> 16) | (b & jnp.uint32(0xFFFF0000))
            dst[2 * pair - base, k:k + kt] = even
            dst[2 * pair - base + 1, k:k + kt] = odd
            yield [even, odd]

    def regroup_rest(i):
        cnt, rem = divmod((3 * H - PRE * GROUP) // 2, PRE - 12)
        assert rem == 0
        for n in range(cnt):
            yield from regroup(PRE * GROUP // 2 + i * cnt + n, False, w1,
                               PRE * GROUP)

    def project_tails(lo, hi, waits, job=lambda i: iter(())):
        for cp in waits:
            cp.wait()

        @pl.loop(0, hi - lo)
        def _(i):
            fresh = [regroup((lo + i) * (GROUP // 2) + n, lo < n_grp, w, 0)
                     for n in range(GROUP // 2)]
            heads = [(lo + i) * GROUP + j for j in range(GROUP)]
            rows = n_seg * 8 // SPLIT
            extra = job(i)
            for n in range(SPLIT):
                y = 0.0
                for k in range(0, D // 2, kt):
                    wk = (sum((next(f) for f in fresh), []) if n == 0 else
                          [w[j, k:k + kt] for j in heads])
                    lhs = ht[n * rows // 2:(n + 1) * rows // 2,
                             2 * k:2 * k + LANES]
                    y += _dot(_unpack([lhs]), _unpack(wk))
                    for _ in range(n_part // SPLIT):
                        next(extra, None)
                for j in range(GROUP):
                    pre[heads[j], n * rows:(n + 1) * rows] = (
                        y[:, j * Dh:(j + 1) * Dh])
            for _ in extra:
                pass

    for cp in cp_tail:
        cp.wait()
    ht[...] = pltpu.bitcast(_layernorm(
        xt[...].astype(F32).reshape(n_seg * 8, D)).astype(BF16), jnp.uint32)
    project_tails(0, 4, cp_q[0])
    project_tails(4, 8, cp_q[1] + cp_filt, transpose_filter)
    project_tails(8, 12, cp_k, gather_filter)
    project_tails(12, PRE, cp_v, regroup_rest)

    for cp in first:
        cp.wait()
    rest = pl.ds(n0, RADIX - n0)
    cp_x = fetch(x_hbm.at[rest], x.at[rest])
    cp_dft = [fetch(fd_hbm, fd), fetch(fs_hbm, fs), fetch(is_hbm, ism),
              fetch(id_hbm, idm)]

    gw = GROUP * Dh

    c1, c2 = math.cos(0.4 * math.pi), math.cos(0.8 * math.pi)
    s1, s2 = math.sin(0.4 * math.pi), math.sin(0.8 * math.pi)
    ch = 16

    def tiles(v):
        return [v[:, c:c + LANES] for c in range(0, v.shape[1], LANES)]

    def fold(s):
        t = tiles(_layernorm(rows_of(s)[...].astype(F32)))
        a1, a2, d1, d2 = t[1] + t[4], t[2] + t[3], t[4] - t[1], t[3] - t[2]
        rows_of(s, fx)[...] = jnp.concatenate(
            [t[0] + a1 + a2,
             t[0] + c1 * a1 + c2 * a2, s1 * d1 + s2 * d2,
             t[0] + c2 * a1 + c1 * a2, s2 * d1 - s1 * d2], axis=1)

    def rows_of(s, ref=x):
        return ref.at[s // per, pl.ds(pl.multiple_of(s % per * seg, seg), seg)]

    def segments(layer, i, mem):
        if layer == 0:
            pl.when(i == 1)(cp_x.wait)
        for n in range(UN_A):
            mem = segment(layer, i * UN_A + n, n % 2, mem)
        return mem

    def segment(layer, s, slot, mem):
        hs = jnp.concatenate([mem, h[slot]], axis=0)
        nxt = rows_of(jnp.minimum(s + 1, n_seg - 1))
        h[1 - slot] = _layernorm(nxt[...].astype(F32))
        fold(jnp.maximum(s - 1, 0))
        row, col = _iota((L, L), 0), _iota((L, L), 1)
        mask = (row < M) | (row >= col)

        tail = pl.ds(pl.multiple_of((s % per * RADIX + s // per) * 8, 8), 8)

        def linear(g):
            heads = range(g * GROUP, (g + 1) * GROUP)
            wg = _unpack([w[j] if g < PRE else w1[j - PRE * GROUP]
                          for j in heads])
            if layer > 0 or g >= PRE:
                return _dot(hs, wg)
            done = jnp.concatenate([pre[j, tail, :] for j in heads], axis=1)
            return jnp.concatenate([_dot(hs[:L - 8], wg), done], axis=0)

        def project(g):
            q, k, v = [linear(t * n_grp + g) for t in range(3)]
            return q, k.astype(BF16), v.astype(BF16)

        def probs(q, k):
            out = []
            for j in range(GROUP):
                c = slice(j * Dh, (j + 1) * Dh)
                sc = jnp.where(mask, _dot_t(q[:, c], k[:, c]) * scale, NEG)
                e = jnp.exp(sc - jnp.max(sc, axis=-1, keepdims=True))
                out.append((e, pltpu.reciprocal(
                    jnp.sum(e, axis=-1, keepdims=True), approx=True)))
            return out

        def attend(ps, v):
            return jnp.concatenate(
                [_dot(e, v[:, j * Dh:(j + 1) * Dh]) * inv
                 for j, (e, inv) in enumerate(ps)], axis=1)

        qkv, ps, os_ = {}, {}, {}
        acc = None
        for t in range(n_grp + 3):
            if t < n_grp:
                qkv[t] = project(t)
            if 0 <= t - 1 < n_grp:
                ps[t - 1] = probs(qkv[t - 1][0], qkv[t - 1][1])
            if 0 <= t - 2 < n_grp:
                os_[t - 2] = attend(ps[t - 2], qkv[t - 2][2])
            if 0 <= t - 3 < n_grp:
                g = t - 3
                y = _dot(os_[g], _unpack(
                    [wo[c, g * gw // 2:(g + 1) * gw // 2, :]
                     for c in range(D // LANES)]))
                acc = y if acc is None else acc + y
        cur = rows_of(s)
        cur[...] = (cur[...].astype(F32) + acc[M:]).astype(BF16)
        return acc[:M]

    def spectral(layer):
        fold(n_seg - 1)

        @pl.loop(0, nb // ch, unroll=UN_D)
        def _(i):
            t = tiles(jnp.concatenate(
                [fx[:, pl.ds(i * ch + o, 8), :].reshape(RADIX * 8, D)
                 for o in range(0, ch, 8)], axis=0))
            o = pl.multiple_of(i * (ch // 2), ch // 2)
            for c, p in enumerate([t[:1], t[1:3], t[3:]]):
                k = len(p) * LANES // 2
                re, im = tiles(_dot(jnp.concatenate(p, axis=1),
                                    _unpack([fd[c, 0, :k], fd[c, 1, :k]])))
                out = [_fft([(re[r:r + 8], im[r:r + 8]) for r in
                             range(n * RADIX * 8, (n + 1) * RADIX * 8, 8)], -1)
                       for n in range(ch // 8)]
                for f1 in range(RADIX):
                    for half in range(2):
                        v = jnp.concatenate([q[f1][half] for q in out], 0)
                        ub[f1, c, pl.ds(o + half * nb // 2, ch // 2), :] = (
                            pltpu.bitcast(v.astype(BF16), jnp.uint32))

        zs = {}
        for t in range(RADIX + LAG):
            if t < RADIX:
                y = _dot(_unpack([fs[t, n] for n in range(fs.shape[1])]),
                         _unpack([ub[t, c] for c in range(nc)]))
                yr, yi = y[:nb], y[nb:]
                wr, wi = filt[t, :, :P], filt[t, :, P:]
                zs[t] = jnp.concatenate(
                    [yr * wr - yi * wi, yr * wi + yi * wr], 0).astype(BF16)
            if t >= LAG:
                f1 = t - LAG
                y = _dot(_unpack([ism[f1, n] for n in range(fs.shape[1])]),
                         zs.pop(f1))
                for c, v in enumerate(tiles(y[:nb]) + tiles(y[nb:])):
                    u[c, f1 * nb:(f1 + 1) * nb, :] = v

        @pl.loop(0, nb // ch, unroll=UN_D)
        def _(i):
            g = []
            for c in range(nc):
                parts = []
                for o in range(0, ch, 8):
                    rows = [pl.ds(f1 * nb + i * ch + o, 8)
                            for f1 in range(RADIX)]
                    out = _fft([(u[c, r, :], u[nc + c, r, :]) for r in rows],
                               1)
                    parts += [jnp.concatenate(v, axis=1) for v in out]
                g += tiles(_dot(jnp.concatenate(parts, axis=0), _unpack(
                    [idm[c, n] for n in range(2 if c else 1)])))
            g0, g1r, g1i, g2r, g2i = g
            a1, a2 = g0 + c1 * g1r + c2 * g2r, g0 + c2 * g1r + c1 * g2r
            b1, b2 = s1 * g1i + s2 * g2i, s2 * g1i - s1 * g2i
            y = jnp.concatenate(
                [g0 + g1r + g2r, a1 - b1, a2 - b2, a2 + b2, a1 + b1], axis=1)
            y = y.reshape(ch // 8, RADIX, 8, D)
            y = jnp.concatenate([y[n] for n in range(ch // 8)], axis=1)
            r = pl.ds(pl.multiple_of(i * ch, ch), ch)
            x[:, r, :] = (x[:, r, :].astype(F32) + y).astype(BF16)

            @pl.when(layer == 1)
            def _():
                pltpu.make_async_copy(x.at[:, r, :], o_hbm.at[:, r, :],
                                      out_sem).start()

    @pl.loop(0, 2)
    def _(layer):
        h[0] = _layernorm(x[0, :seg, :].astype(F32))
        for n in range(2):
            @pl.when(layer == n)
            def _():
                jax.lax.fori_loop(0, n_seg // UN_A,
                                  functools.partial(segments, n),
                                  memb[...].astype(F32))
                if n == 0:
                    for cp in cp_dft:
                        cp.wait()

        spectral(layer)

    pltpu.make_async_copy(x, o_hbm, out_sem).wait()


@functools.partial(jax.jit, static_argnames=("A_seg_len",))
def pallas_interleave_layers__memory_aug_recurrent_mem_tr__spectral_gfnet__prompt_kernel(
    A_x, A_mem0, A_Wq, A_Wk, A_Wv, A_Wo, A_seg_len, B_x, B_w_r, B_w_i,
):
    del B_x
    B, S, D = A_x.shape
    _, H, Dh = A_Wq.shape
    M = A_mem0.shape[1]
    assert B == 1 and Dh == LANES and D == 5 * LANES
    consts = _dft_constants(S, D)
    n_seg = S // A_seg_len
    per = n_seg // RADIX
    args = [A_x.reshape(RADIX, S // RADIX, D), A_mem0.reshape(M, D),
            A_Wq.reshape(D // 2, 2 * H, Dh), A_Wk.reshape(D // 2, 2 * H, Dh),
            A_Wv.reshape(D // 2, 2 * H, Dh), A_Wo.reshape(H * Dh, D),
            B_w_r.T, B_w_i.T] + consts
    u32 = jnp.uint32
    out = pl.pallas_call(
        functools.partial(_kernel, S=S, D=D, H=H, Dh=Dh, M=M, seg=A_seg_len),
        out_shape=jax.ShapeDtypeStruct((RADIX, S // RADIX, D), BF16),
        in_specs=[pl.BlockSpec(memory_space=pltpu.HBM)] * len(args),
        out_specs=pl.BlockSpec(memory_space=pltpu.HBM),
        scratch_shapes=[
            pltpu.VMEM((RADIX, S // RADIX, D), BF16),
            pltpu.VMEM((M, D), BF16),
            pltpu.VMEM((4, D // 2 * (H // 4), Dh), u32),
            pltpu.VMEM((4, D // 2 * (H // 2 + 8), Dh), u32),
            pltpu.VMEM((PRE * GROUP, D // 2, Dh), u32),
            pltpu.VMEM((3 * H - PRE * GROUP, D // 2, Dh), u32),
            pltpu.VMEM((D // LANES, H * Dh // 2, LANES), u32),
            pltpu.VMEM(B_w_r.shape[::-1], BF16),
            pltpu.VMEM(B_w_i.shape[::-1], BF16),
        ] + [pltpu.VMEM(c.shape, u32) for c in consts] + [
            pltpu.VMEM((S // LANES // 2, 3 * LANES, LANES), F32),
            pltpu.VMEM((per, RADIX, 8, D), BF16),
            pltpu.VMEM((n_seg * 4, D), u32),
            pltpu.VMEM((PRE * GROUP, n_seg * 8, Dh), F32),
            pltpu.VMEM((2, A_seg_len, D), F32),
            pltpu.VMEM((RADIX, S // RADIX, D), F32),
            pltpu.VMEM((RADIX, 3, S // RADIX, LANES), u32),
            pltpu.VMEM((6, S // RADIX * (RADIX + 8), LANES), F32),
            pltpu.VMEM((RADIX, S // RADIX, 6 * LANES), F32),
            pltpu.SemaphoreType.DMA((17 + D // LANES + per,)),
            pltpu.SemaphoreType.DMA(()),
        ],
        compiler_params=pltpu.CompilerParams(vmem_limit_bytes=110 * 2 ** 20),
    )(*args)
    return out.reshape(B, S, D)
```

```python
import functools
import math

import jax
import jax.numpy as jnp
import numpy as np
import jax.experimental.pallas as pl
import jax.experimental.pallas.tpu as pltpu

F32 = jnp.float32
BF16 = jnp.bfloat16
LANES = 128
RADIX = 32
GROUP = 4
LAG = 2
SPLIT = 4
PRE = 14
UN_A = 2
EPS = 1e-5
NEG = -1000000000.0


def _pack(a):
    bits = a.astype(np.float32).astype(BF16).view(np.uint16).astype(np.uint32)
    words = bits[..., 0::2, :] | (bits[..., 1::2, :] << 16)
    words = words.reshape(words.shape[:-1] + (-1, LANES))
    return np.ascontiguousarray(np.swapaxes(words, -2, -3))


def _dft_constants(S, D):
    j = np.arange(LANES)
    b = j[:, None]
    fwd_d, inv_d = [], []
    for k1 in range(3):
        k = np.where(j < 64, k1 + 5 * j, D - (5 - k1) - 5 * (j - 64))
        wgt = np.full((LANES,), 2.0)
        if k1 == 0:
            k = 5 * j
            wgt = np.where(j < 64, 2.0, 0.0)
            wgt[0] = wgt[64] = 1.0
        ang = 2.0 * np.pi * ((b * k) % D) / D
        c, s = np.cos(ang), np.sin(ang)
        s[:, (2 * k) % D == 0] = 0.0
        m = np.block([[c, -s], [s, c]])
        fwd_d.append(m)
        inv_d.append(m.T * np.tile(wgt, 2)[:, None] / D)
    j = np.arange(S // RADIX)
    f = np.arange(RADIX)[:, None, None] + RADIX * j[None, :, None]
    ang = 2.0 * np.pi * ((j[None, None, :] * f) % S) / S
    c, s = np.cos(ang), np.sin(ang)
    fwd_s = np.concatenate([np.concatenate([c, s], 2),
                            np.concatenate([-s, c], 2)], 1)
    inv_s = np.swapaxes(fwd_s, 1, 2) / S
    return [_pack(a) for a in (np.stack(fwd_d), np.stack(inv_d), fwd_s, inv_s)]


def _twiddle(v, j, n, sign):
    pr, pi = v
    c = math.cos(2 * math.pi * j / n)
    s = sign * math.sin(2 * math.pi * j / n)
    if j == 0:
        return v
    if 4 * j == n:
        return (-pi, pr) if sign > 0 else (pi, -pr)
    if 8 * j % n == 0:
        return (((pr - pi) * c, (pr + pi) * c) if c * s > 0 else
                ((pr + pi) * c, (pi - pr) * c))
    return pr * c - pi * s, pr * s + pi * c


def _fft(vals, sign):
    n = len(vals)
    if n == 1:
        return [vals[0]()]
    ev, od = _fft(vals[0::2], sign), _fft(vals[1::2], sign)
    lo, hi = [], []
    for j in range(n // 2):
        er, ei = ev[j]
        if 4 * j == n:
            pr, pi = od[j]
            a, b = (er - pi, ei + pr), (er + pi, ei - pr)
            lo.append(a if sign > 0 else b)
            hi.append(b if sign > 0 else a)
        else:
            pr, pi = _twiddle(od[j], j, n, sign)
            lo.append((er + pr, ei + pi))
            hi.append((er - pr, ei - pi))
    return lo + hi


def _dot(a, b):
    return jax.lax.dot_general(a, b, (((1,), (0,)), ((), ())),
                               preferred_element_type=F32)


def _dot_t(a, b):
    return jax.lax.dot_general(a, b, (((1,), (1,)), ((), ())),
                               preferred_element_type=F32)


def _unpack(tiles):
    return pltpu.bitcast(jnp.concatenate(tiles, axis=1), BF16)


def _layernorm(x):
    xc = x - jnp.mean(x, axis=-1, keepdims=True)
    var = jnp.mean(xc * xc, axis=-1, keepdims=True)
    return xc * jax.lax.rsqrt(var + EPS)


def _iota(shape, axis):
    return jax.lax.broadcasted_iota(jnp.int32, shape, axis)


def _kernel(x_hbm, mem_hbm, wq_hbm, wk_hbm, wv_hbm, wo_hbm, wr_hbm, wi_hbm,
            fd_hbm, id_hbm, fs_hbm, is_hbm, o_hbm,
            x, memb, stage_q, stage, w, w1, wo, wrb, wib, fd, idm, fs, ism,
            tmp, xt, ht, pre, h, fx, ub, u, filt, sems, out_sem, *, S, D, H, Dh, M, seg):
    L = M + seg
    n_seg = S // seg
    nb = S // RADIX
    nc = 3
    P = nc * LANES
    Df = wrb.shape[0]
    scale = Dh ** -0.5

    started = []

    def fetch(src, dst):
        cp = pltpu.make_async_copy(src, dst, sems.at[len(started)])
        cp.start()
        started.append(cp)
        return cp

    per = nb // seg

    def fetch_w(src, buf, slot, lo, n):
        pitch = buf.shape[1] // (D // 2)
        return [fetch(
            src.bitcast(jnp.uint32).at[:, pl.ds(par * H // 2 + lo, n)],
            buf.at[2 * slot + par].reshape(D // 2, pitch, Dh)
            .at[:, pl.ds(0, n)]) for par in range(2)]

    cp_tail = [fetch(x_hbm.at[:, pl.ds((n + 1) * seg - 8, 8)], xt.at[n])
               for n in range(per)]
    cp_q = [fetch_w(wq_hbm, stage_q, n, n * H // 4, H // 4) for n in range(2)]
    cp_filt = [fetch(wr_hbm, wrb), fetch(wi_hbm, wib)]
    cp_k = fetch_w(wk_hbm, stage, 0, 0, H // 2)
    cp_v = fetch_w(wv_hbm, stage, 1, 0, H // 2)
    n0 = pl.cdiv((UN_A + 1) * seg, nb)
    first = [fetch(mem_hbm, memb), fetch(x_hbm.at[:n0], x.at[:n0])]
    first += [fetch(wo_hbm.bitcast(jnp.uint32).at[:, pl.ds(c * LANES, LANES)],
                    wo.at[c])
              for c in range(D // LANES)]

    n_part = tmp.shape[0]
    gap = RADIX + 8

    def transpose_filter(i):
        for n in range(n_part):
            blk = i * (n_part // 2) + n // 2
            r = pl.ds(pl.multiple_of(blk * LANES, LANES), LANES)
            tmp[n] = jnp.concatenate(
                [(wrb, wib)[n % 2][:, r].astype(F32),
                 jnp.zeros((P - Df, LANES), F32)], 0)
            yield
            for c in range(nc):
                v = jnp.concatenate(
                    [tmp[n, pl.ds(c, 64 if c else 72, stride=5), :],
                     tmp[n, pl.ds(5 - c, 64, stride=5), :] if c
                     else jnp.zeros((56, LANES), F32)], axis=0).T
                for m in range(LANES // RADIX):
                    o = pl.multiple_of((blk * (LANES // RADIX) + m) * gap, 8)
                    u[n % 2 * nc + c, pl.ds(o, RADIX), :] = (
                        v[m * RADIX:(m + 1) * RADIX])
                yield

    def gather_filter(i):
        for n in range(n_part):
            f1 = i * n_part + n
            pos = _iota((nb, nb), 0) + _iota((nb, nb), 1) + jnp.minimum(f1, 1)
            flip = jnp.where((pos == 0) | (pos == nb), 1.0, 0.0)
            neg = pl.ds((RADIX - f1) % RADIX, nb, stride=gap)
            mixed = [c for c in range(2 * nc) if c % nc]
            m = _dot(flip, jnp.concatenate(
                [u[c, neg, :] for c in mixed], axis=1).astype(BF16))
            yield
            yield
            for c in range(2 * nc):
                v = u[c, pl.ds(f1, nb, stride=gap), :]
                if c % nc:
                    o = mixed.index(c) * LANES
                    mc = m[:, o:o + LANES]
                    v = jnp.where(_iota((nb, LANES), 1) < 64, v,
                                  mc if c < nc else -mc)
                filt[f1, :, c * LANES:(c + 1) * LANES] = v
                if c % 2:
                    yield

    n_grp = H // GROUP
    kt = LANES // 2

    def regroup(pair, is_q, dst, base):
        buf, n, q = ((stage_q, H // 4, pair) if is_q else
                     (stage, H // 2, pair - H // 2))
        pitch = buf.shape[1] // (D // 2)
        for k in range(0, D // 2, kt):
            j = pl.ds(q % n + k * pitch, kt, stride=pitch)
            a, b = [buf[q // n * 2 + par, j, :] for par in range(2)]
            even = (a & jnp.uint32(0xFFFF)) | (b << 16)
            odd = (a >> 16) | (b & jnp.uint32(0xFFFF0000))
            dst[2 * pair - base, k:k + kt] = even
            dst[2 * pair - base + 1, k:k + kt] = odd
            yield [even, odd]

    def regroup_rest(i):
        cnt, rem = divmod((3 * H - PRE * GROUP) // 2, PRE - 12)
        assert rem == 0
        for n in range(cnt):
            yield from regroup(PRE * GROUP // 2 + i * cnt + n, False, w1,
                               PRE * GROUP)

    def project_tails(lo, hi, waits, job=lambda i: iter(())):
        for cp in waits:
            cp.wait()

        @pl.loop(0, hi - lo)
        def _(i):
            fresh = [regroup((lo + i) * (GROUP // 2) + n, lo < n_grp, w, 0)
                     for n in range(GROUP // 2)]
            heads = [(lo + i) * GROUP + j for j in range(GROUP)]
            rows = n_seg * 8 // SPLIT
            extra = job(i)
            for n in range(SPLIT):
                y = 0.0
                for k in range(0, D // 2, kt):
                    wk = (sum((next(f) for f in fresh), []) if n == 0 else
                          [w[j, k:k + kt] for j in heads])
                    lhs = ht[n * rows // 2:(n + 1) * rows // 2,
                             2 * k:2 * k + LANES]
                    y += _dot(_unpack([lhs]), _unpack(wk))
                    for _ in range(n_part // SPLIT):
                        next(extra, None)
                for j in range(GROUP):
                    pre[heads[j], n * rows:(n + 1) * rows] = (
                        y[:, j * Dh:(j + 1) * Dh])
            for _ in extra:
                pass

    for cp in cp_tail:
        cp.wait()
    ht[...] = pltpu.bitcast(_layernorm(
        xt[...].astype(F32).reshape(n_seg * 8, D)).astype(BF16), jnp.uint32)
    project_tails(0, 4, cp_q[0])
    project_tails(4, 8, cp_q[1] + cp_filt, transpose_filter)
    project_tails(8, 12, cp_k, gather_filter)
    project_tails(12, PRE, cp_v, regroup_rest)

    for cp in first:
        cp.wait()
    rest = pl.ds(n0, RADIX - n0)
    cp_x = fetch(x_hbm.at[rest], x.at[rest])
    cp_dft = [fetch(fd_hbm, fd), fetch(fs_hbm, fs), fetch(is_hbm, ism),
              fetch(id_hbm, idm)]

    gw = GROUP * Dh

    c1, c2 = math.cos(0.4 * math.pi), math.cos(0.8 * math.pi)
    s1, s2 = math.sin(0.4 * math.pi), math.sin(0.8 * math.pi)
    ch = 16

    def tiles(v):
        return [v[:, c:c + LANES] for c in range(0, v.shape[1], LANES)]

    def fold(s):
        t = tiles(_layernorm(rows_of(s)[...].astype(F32)))
        a1, a2, d1, d2 = t[1] + t[4], t[2] + t[3], t[4] - t[1], t[3] - t[2]
        rows_of(s, fx)[...] = jnp.concatenate(
            [t[0] + a1 + a2,
             t[0] + c1 * a1 + c2 * a2, s1 * d1 + s2 * d2,
             t[0] + c2 * a1 + c1 * a2, s2 * d1 - s1 * d2], axis=1)

    def rows_of(s, ref=x):
        return ref.at[s // per, pl.ds(pl.multiple_of(s % per * seg, seg), seg)]

    def segments(layer, i, mem):
        if layer == 0:
            pl.when(i == 1)(cp_x.wait)
        for n in range(UN_A):
            mem = segment(layer, i * UN_A + n, n % 2, mem)
        return mem

    def segment(layer, s, slot, mem):
        hs = jnp.concatenate([mem, h[slot]], axis=0)
        nxt = rows_of(jnp.minimum(s + 1, n_seg - 1))
        h[1 - slot] = _layernorm(nxt[...].astype(F32))
        fold(jnp.maximum(s - 1, 0))
        row, col = _iota((L, L), 0), _iota((L, L), 1)
        mask = (row < M) | (row >= col)

        tail = pl.ds(pl.multiple_of((s % per * RADIX + s // per) * 8, 8), 8)

        def linear(g):
            heads = range(g * GROUP, (g + 1) * GROUP)
            wg = _unpack([w[j] if g < PRE else w1[j - PRE * GROUP]
                          for j in heads])
            if layer > 0 or g >= PRE:
                return _dot(hs, wg)
            done = jnp.concatenate([pre[j, tail, :] for j in heads], axis=1)
            return jnp.concatenate([_dot(hs[:L - 8], wg), done], axis=0)

        def project(g):
            q, k, v = [linear(t * n_grp + g) for t in range(3)]
            return q, k.astype(BF16), v.astype(BF16)

        def probs(q, k):
            out = []
            for j in range(GROUP):
                c = slice(j * Dh, (j + 1) * Dh)
                sc = jnp.where(mask, _dot_t(q[:, c], k[:, c]) * scale, NEG)
                e = jnp.exp(sc - jnp.max(sc, axis=-1, keepdims=True))
                out.append((e, pltpu.reciprocal(
                    jnp.sum(e, axis=-1, keepdims=True), approx=True)))
            return out

        def attend(ps, v):
            return jnp.concatenate(
                [_dot(e, v[:, j * Dh:(j + 1) * Dh]) * inv
                 for j, (e, inv) in enumerate(ps)], axis=1)

        qkv, ps, os_ = {}, {}, {}
        acc = None
        for t in range(n_grp + 3):
            if t < n_grp:
                qkv[t] = project(t)
            if 0 <= t - 1 < n_grp:
                ps[t - 1] = probs(qkv[t - 1][0], qkv[t - 1][1])
            if 0 <= t - 2 < n_grp:
                os_[t - 2] = attend(ps[t - 2], qkv[t - 2][2])
            if 0 <= t - 3 < n_grp:
                g = t - 3
                y = _dot(os_[g], _unpack(
                    [wo[c, g * gw // 2:(g + 1) * gw // 2, :]
                     for c in range(D // LANES)]))
                acc = y if acc is None else acc + y
        cur = rows_of(s)
        cur[...] = (cur[...].astype(F32) + acc[M:]).astype(BF16)
        return acc[:M]

    def spectral(layer):
        fold(n_seg - 1)

        hr = RADIX // 2
        for i in range(0, nb, ch):
            for odd in range(2):
                halves = []
                for o in range(i, i + ch, 8):
                    lo, hi = fx[:hr, o:o + 8, :], fx[hr:, o:o + 8, :]
                    halves.append((lo - hi if odd else lo + hi)
                                  .reshape(hr * 8, D))
                t = tiles(jnp.concatenate(halves, axis=0))
                for c, p in enumerate([t[:1], t[1:3], t[3:]]):
                    k = len(p) * kt
                    re, im = tiles(_dot(
                        jnp.concatenate(p, axis=1),
                        _unpack([fd[c, 0, :k], fd[c, 1, :k]])))

                    def term(n, a):
                        r = slice((n * hr + a) * 8, (n * hr + a + 1) * 8)
                        return _twiddle((re[r], im[r]), a * odd, RADIX, -1)

                    out = [_fft([functools.partial(term, n, a)
                                 for a in range(hr)], -1)
                           for n in range(ch // 8)]
                    for f in range(hr):
                        for half in range(2):
                            v = jnp.concatenate([q[f][half] for q in out], 0)
                            r = pl.ds((i + half * nb) // 2, ch // 2)
                            ub[2 * f + odd, c, r, :] = pltpu.bitcast(
                                v.astype(BF16), jnp.uint32)

        zs = {}
        for t in range(RADIX + LAG):
            if t < RADIX:
                y = _dot(_unpack([fs[t, n] for n in range(fs.shape[1])]),
                         _unpack([ub[t, c] for c in range(nc)]))
                yr, yi = y[:nb], y[nb:]
                wr, wi = filt[t, :, :P], filt[t, :, P:]
                zs[t] = jnp.concatenate(
                    [yr * wr - yi * wi, yr * wi + yi * wr], 0).astype(BF16)
            if t >= LAG:
                f1 = t - LAG
                y = _dot(_unpack([ism[f1, n] for n in range(fs.shape[1])]),
                         zs.pop(f1))
                for c, v in enumerate(tiles(y[:nb]) + tiles(y[nb:])):
                    u[c, f1 * nb:(f1 + 1) * nb, :] = v

        for i in range(0, nb, ch):
            r = pl.ds(i, ch)
            for odd in range(2):
                ys = []
                for o in range(i, i + ch, 8):
                    def term(c, f):
                        lo, hi = [[u[c + h_, pl.ds(f_ * nb + o, 8), :]
                                   for h_ in (0, nc)] for f_ in (f, f + hr)]
                        v = [p - q if odd else p + q for p, q in zip(lo, hi)]
                        return _twiddle(v, f * odd, RADIX, 1)

                    g = []
                    for c in range(nc):
                        out = _fft([functools.partial(term, c, f)
                                    for f in range(hr)], 1)
                        z = jnp.concatenate(
                            [jnp.concatenate(v, axis=1) for v in out], axis=0)
                        g += tiles(_dot(z, _unpack(
                            [idm[c, n] for n in range(2 if c else 1)])))
                    g0, g1r, g1i, g2r, g2i = g
                    a1 = g0 + c1 * g1r + c2 * g2r
                    a2 = g0 + c2 * g1r + c1 * g2r
                    b1, b2 = s1 * g1i + s2 * g2i, s2 * g1i - s1 * g2i
                    ys.append(jnp.concatenate(
                        [g0 + g1r + g2r, a1 - b1, a2 - b2, a2 + b2, a1 + b1],
                        axis=1))
                for a in range(hr):
                    y = jnp.concatenate([v[a * 8:a * 8 + 8] for v in ys], 0)
                    x[2 * a + odd, r, :] = (
                        x[2 * a + odd, r, :].astype(F32) + y).astype(BF16)

            @pl.when(layer == 1)
            def _():
                pltpu.make_async_copy(x.at[:, r, :], o_hbm.at[:, r, :],
                                      out_sem).start()

    @pl.loop(0, 2)
    def _(layer):
        h[0] = _layernorm(x[0, :seg, :].astype(F32))
        for n in range(2):
            @pl.when(layer == n)
            def _():
                jax.lax.fori_loop(0, n_seg // UN_A,
                                  functools.partial(segments, n),
                                  memb[...].astype(F32))
                if n == 0:
                    for cp in cp_dft:
                        cp.wait()

        spectral(layer)

    pltpu.make_async_copy(x, o_hbm, out_sem).wait()


@functools.partial(jax.jit, static_argnames=("A_seg_len",))
def pallas_interleave_layers__memory_aug_recurrent_mem_tr__spectral_gfnet__prompt_kernel(
    A_x, A_mem0, A_Wq, A_Wk, A_Wv, A_Wo, A_seg_len, B_x, B_w_r, B_w_i,
):
    del B_x
    B, S, D = A_x.shape
    _, H, Dh = A_Wq.shape
    M = A_mem0.shape[1]
    assert B == 1 and Dh == LANES and D == 5 * LANES
    consts = _dft_constants(S, D)
    n_seg = S // A_seg_len
    per = n_seg // RADIX
    args = [A_x.reshape(RADIX, S // RADIX, D), A_mem0.reshape(M, D),
            A_Wq.reshape(D // 2, 2 * H, Dh), A_Wk.reshape(D // 2, 2 * H, Dh),
            A_Wv.reshape(D // 2, 2 * H, Dh), A_Wo.reshape(H * Dh, D),
            B_w_r.T, B_w_i.T] + consts
    u32 = jnp.uint32
    out = pl.pallas_call(
        functools.partial(_kernel, S=S, D=D, H=H, Dh=Dh, M=M, seg=A_seg_len),
        out_shape=jax.ShapeDtypeStruct((RADIX, S // RADIX, D), BF16),
        in_specs=[pl.BlockSpec(memory_space=pltpu.HBM)] * len(args),
        out_specs=pl.BlockSpec(memory_space=pltpu.HBM),
        scratch_shapes=[
            pltpu.VMEM((RADIX, S // RADIX, D), BF16),
            pltpu.VMEM((M, D), BF16),
            pltpu.VMEM((4, D // 2 * (H // 4), Dh), u32),
            pltpu.VMEM((4, D // 2 * (H // 2 + 8), Dh), u32),
            pltpu.VMEM((PRE * GROUP, D // 2, Dh), u32),
            pltpu.VMEM((3 * H - PRE * GROUP, D // 2, Dh), u32),
            pltpu.VMEM((D // LANES, H * Dh // 2, LANES), u32),
            pltpu.VMEM(B_w_r.shape[::-1], BF16),
            pltpu.VMEM(B_w_i.shape[::-1], BF16),
        ] + [pltpu.VMEM(c.shape, u32) for c in consts] + [
            pltpu.VMEM((S // LANES // 2, 3 * LANES, LANES), F32),
            pltpu.VMEM((per, RADIX, 8, D), BF16),
            pltpu.VMEM((n_seg * 4, D), u32),
            pltpu.VMEM((PRE * GROUP, n_seg * 8, Dh), F32),
            pltpu.VMEM((2, A_seg_len, D), F32),
            pltpu.VMEM((RADIX, S // RADIX, D), F32),
            pltpu.VMEM((RADIX, 3, S // RADIX, LANES), u32),
            pltpu.VMEM((6, S // RADIX * (RADIX + 8), LANES), F32),
            pltpu.VMEM((RADIX, S // RADIX, 6 * LANES), F32),
            pltpu.SemaphoreType.DMA((17 + D // LANES + per,)),
            pltpu.SemaphoreType.DMA(()),
        ],
        compiler_params=pltpu.CompilerParams(vmem_limit_bytes=110 * 2 ** 20),
    )(*args)
    return out.reshape(B, S, D)
```

```python
import functools
import math

import jax
import jax.numpy as jnp
import numpy as np
import jax.experimental.pallas as pl
import jax.experimental.pallas.tpu as pltpu

F32 = jnp.float32
BF16 = jnp.bfloat16
LANES = 128
RADIX = 32
GROUP = 4
SPLIT = 4
PRE = 14
UN_A = 2
EPS = 1e-5
NEG = -1000000000.0


def _pack(a):
    bits = a.astype(np.float32).astype(BF16).view(np.uint16).astype(np.uint32)
    words = bits[..., 0::2, :] | (bits[..., 1::2, :] << 16)
    words = words.reshape(words.shape[:-1] + (-1, LANES))
    return np.ascontiguousarray(np.swapaxes(words, -2, -3))


def _dft_constants(S, D):
    j = np.arange(LANES)
    b = j[:, None]
    fwd_d, inv_d = [], []
    for k1 in range(3):
        k = np.where(j < 64, k1 + 5 * j, D - (5 - k1) - 5 * (j - 64))
        wgt = np.full((LANES,), 2.0)
        if k1 == 0:
            k = 5 * j
            wgt = np.where(j < 64, 2.0, 0.0)
            wgt[0] = wgt[64] = 1.0
        ang = 2.0 * np.pi * ((b * k) % D) / D
        c, s = np.cos(ang), np.sin(ang)
        s[:, (2 * k) % D == 0] = 0.0
        m = np.block([[c, -s], [s, c]])
        fwd_d.append(m)
        inv_d.append(m.T * np.tile(wgt, 2)[:, None] / D)
    j = np.arange(S // RADIX)
    f = np.arange(RADIX)[:, None, None] + RADIX * j[None, :, None]
    ang = 2.0 * np.pi * ((j[None, None, :] * f) % S) / S
    c, s = np.cos(ang), np.sin(ang)
    fwd_s = np.concatenate([np.concatenate([c, s], 2),
                            np.concatenate([-s, c], 2)], 1)
    inv_s = np.swapaxes(fwd_s, 1, 2) / S
    return [_pack(a) for a in (np.stack(fwd_d), np.stack(inv_d), fwd_s, inv_s)]


def _twiddle(v, j, n, sign):
    pr, pi = v
    c = math.cos(2 * math.pi * j / n)
    s = sign * math.sin(2 * math.pi * j / n)
    if j == 0:
        return v
    if 4 * j == n:
        return (-pi, pr) if sign > 0 else (pi, -pr)
    if 8 * j % n == 0:
        return (((pr - pi) * c, (pr + pi) * c) if c * s > 0 else
                ((pr + pi) * c, (pi - pr) * c))
    return pr * c - pi * s, pr * s + pi * c


def _fft(vals, sign):
    n = len(vals)
    if n == 1:
        return [vals[0]()]
    ev, od = _fft(vals[0::2], sign), _fft(vals[1::2], sign)
    lo, hi = [], []
    for j in range(n // 2):
        er, ei = ev[j]
        if 4 * j == n:
            pr, pi = od[j]
            a, b = (er - pi, ei + pr), (er + pi, ei - pr)
            lo.append(a if sign > 0 else b)
            hi.append(b if sign > 0 else a)
        else:
            pr, pi = _twiddle(od[j], j, n, sign)
            lo.append((er + pr, ei + pi))
            hi.append((er - pr, ei - pi))
    return lo + hi


def _dot(a, b):
    return jax.lax.dot_general(a, b, (((1,), (0,)), ((), ())),
                               preferred_element_type=F32)


def _dot_t(a, b):
    return jax.lax.dot_general(a, b, (((1,), (1,)), ((), ())),
                               preferred_element_type=F32)


def _unpack(tiles):
    return pltpu.bitcast(jnp.concatenate(tiles, axis=1), BF16)


def _layernorm(x):
    xc = x - jnp.mean(x, axis=-1, keepdims=True)
    var = jnp.mean(xc * xc, axis=-1, keepdims=True)
    return xc * jax.lax.rsqrt(var + EPS)


def _iota(shape, axis):
    return jax.lax.broadcasted_iota(jnp.int32, shape, axis)


def _kernel(x_hbm, mem_hbm, wq_hbm, wk_hbm, wv_hbm, wo_hbm, wr_hbm, wi_hbm,
            fd_hbm, id_hbm, fs_hbm, is_hbm, o_hbm,
            x, memb, stage_q, stage, w, w1, wo, wrb, wib, fd, idm, fs, ism,
            tmp, xt, ht, pre, h, fx, ub, u, filt, sems, out_sem, *, S, D, H, Dh, M, seg):
    L = M + seg
    n_seg = S // seg
    nb = S // RADIX
    nc = 3
    P = nc * LANES
    Df = wrb.shape[0]
    scale = Dh ** -0.5

    started = []

    def fetch(src, dst):
        cp = pltpu.make_async_copy(src, dst, sems.at[len(started)])
        cp.start()
        started.append(cp)
        return cp

    per = nb // seg

    def fetch_w(src, buf, slot, lo, n):
        pitch = buf.shape[1] // (D // 2)
        return [fetch(
            src.bitcast(jnp.uint32).at[:, pl.ds(par * H // 2 + lo, n)],
            buf.at[2 * slot + par].reshape(D // 2, pitch, Dh)
            .at[:, pl.ds(0, n)]) for par in range(2)]

    cp_tail = [fetch(x_hbm.at[:, pl.ds((n + 1) * seg - 8, 8)], xt.at[n])
               for n in range(per)]
    cp_q = [fetch_w(wq_hbm, stage_q, n, n * H // 4, H // 4) for n in range(2)]
    cp_filt = [fetch(wr_hbm, wrb), fetch(wi_hbm, wib)]
    cp_k = fetch_w(wk_hbm, stage, 0, 0, H // 2)
    cp_v = fetch_w(wv_hbm, stage, 1, 0, H // 2)
    n0 = pl.cdiv((UN_A + 1) * seg, nb)
    first = [fetch(mem_hbm, memb), fetch(x_hbm.at[:n0], x.at[:n0])]
    first += [fetch(wo_hbm.bitcast(jnp.uint32).at[:, pl.ds(c * LANES, LANES)],
                    wo.at[c])
              for c in range(D // LANES)]

    n_part = tmp.shape[0]
    gap = RADIX + 8

    def transpose_filter(i):
        for n in range(n_part):
            blk = i * (n_part // 2) + n // 2
            r = pl.ds(pl.multiple_of(blk * LANES, LANES), LANES)
            tmp[n] = jnp.concatenate(
                [(wrb, wib)[n % 2][:, r].astype(F32),
                 jnp.zeros((P - Df, LANES), F32)], 0)
            yield
            for c in range(nc):
                v = jnp.concatenate(
                    [tmp[n, pl.ds(c, 64 if c else 72, stride=5), :],
                     tmp[n, pl.ds(5 - c, 64, stride=5), :] if c
                     else jnp.zeros((56, LANES), F32)], axis=0).T
                for m in range(LANES // RADIX):
                    o = pl.multiple_of((blk * (LANES // RADIX) + m) * gap, 8)
                    u[n % 2 * nc + c, pl.ds(o, RADIX), :] = (
                        v[m * RADIX:(m + 1) * RADIX])
                yield

    def gather_filter(i):
        for n in range(n_part):
            f1 = i * n_part + n
            pos = _iota((nb, nb), 0) + _iota((nb, nb), 1) + jnp.minimum(f1, 1)
            flip = jnp.where((pos == 0) | (pos == nb), 1.0, 0.0)
            neg = pl.ds((RADIX - f1) % RADIX, nb, stride=gap)
            mixed = [c for c in range(2 * nc) if c % nc]
            m = _dot(flip, jnp.concatenate(
                [u[c, neg, :] for c in mixed], axis=1).astype(BF16))
            yield
            yield
            for c in range(2 * nc):
                v = u[c, pl.ds(f1, nb, stride=gap), :]
                if c % nc:
                    o = mixed.index(c) * LANES
                    mc = m[:, o:o + LANES]
                    v = jnp.where(_iota((nb, LANES), 1) < 64, v,
                                  mc if c < nc else -mc)
                filt[f1, :, c * LANES:(c + 1) * LANES] = v
                if c % 2:
                    yield

    n_grp = H // GROUP
    kt = LANES // 2

    def regroup(pair, is_q, dst, base):
        buf, n, q = ((stage_q, H // 4, pair) if is_q else
                     (stage, H // 2, pair - H // 2))
        pitch = buf.shape[1] // (D // 2)
        for k in range(0, D // 2, kt):
            j = pl.ds(q % n + k * pitch, kt, stride=pitch)
            a, b = [buf[q // n * 2 + par, j, :] for par in range(2)]
            even = (a & jnp.uint32(0xFFFF)) | (b << 16)
            odd = (a >> 16) | (b & jnp.uint32(0xFFFF0000))
            dst[2 * pair - base, k:k + kt] = even
            dst[2 * pair - base + 1, k:k + kt] = odd
            yield [even, odd]

    def regroup_rest(i):
        cnt, rem = divmod((3 * H - PRE * GROUP) // 2, PRE - 12)
        assert rem == 0
        for n in range(cnt):
            yield from regroup(PRE * GROUP // 2 + i * cnt + n, False, w1,
                               PRE * GROUP)

    def project_tails(lo, hi, waits, job=lambda i: iter(())):
        for cp in waits:
            cp.wait()

        @pl.loop(0, hi - lo)
        def _(i):
            fresh = [regroup((lo + i) * (GROUP // 2) + n, lo < n_grp, w, 0)
                     for n in range(GROUP // 2)]
            heads = [(lo + i) * GROUP + j for j in range(GROUP)]
            rows = n_seg * 8 // SPLIT
            extra = job(i)
            for n in range(SPLIT):
                y = 0.0
                for k in range(0, D // 2, kt):
                    wk = (sum((next(f) for f in fresh), []) if n == 0 else
                          [w[j, k:k + kt] for j in heads])
                    lhs = ht[n * rows // 2:(n + 1) * rows // 2,
                             2 * k:2 * k + LANES]
                    y += _dot(_unpack([lhs]), _unpack(wk))
                    for _ in range(n_part // SPLIT):
                        next(extra, None)
                for j in range(GROUP):
                    pre[heads[j], n * rows:(n + 1) * rows] = (
                        y[:, j * Dh:(j + 1) * Dh])
            for _ in extra:
                pass

    for cp in cp_tail:
        cp.wait()
    ht[...] = pltpu.bitcast(_layernorm(
        xt[...].astype(F32).reshape(n_seg * 8, D)).astype(BF16), jnp.uint32)
    project_tails(0, 4, cp_q[0])
    project_tails(4, 8, cp_q[1] + cp_filt, transpose_filter)
    project_tails(8, 12, cp_k, gather_filter)
    project_tails(12, PRE, cp_v, regroup_rest)

    for cp in first:
        cp.wait()
    rest = pl.ds(n0, RADIX - n0)
    cp_x = fetch(x_hbm.at[rest], x.at[rest])
    cp_dft = [fetch(fd_hbm, fd), fetch(fs_hbm, fs), fetch(is_hbm, ism),
              fetch(id_hbm, idm)]

    gw = GROUP * Dh

    c1, c2 = math.cos(0.4 * math.pi), math.cos(0.8 * math.pi)
    s1, s2 = math.sin(0.4 * math.pi), math.sin(0.8 * math.pi)
    ch = 16

    def tiles(v):
        return [v[:, c:c + LANES] for c in range(0, v.shape[1], LANES)]

    def fold(s):
        t = tiles(_layernorm(rows_of(s)[...].astype(F32)))
        a1, a2, d1, d2 = t[1] + t[4], t[2] + t[3], t[4] - t[1], t[3] - t[2]
        rows_of(s, fx)[...] = jnp.concatenate(
            [t[0] + a1 + a2,
             t[0] + c1 * a1 + c2 * a2, s1 * d1 + s2 * d2,
             t[0] + c2 * a1 + c1 * a2, s2 * d1 - s1 * d2], axis=1)

    def rows_of(s, ref=x):
        return ref.at[s // per, pl.ds(pl.multiple_of(s % per * seg, seg), seg)]

    def segments(layer, i, mem):
        if layer == 0:
            pl.when(i == 1)(cp_x.wait)
        for n in range(UN_A):
            mem = segment(layer, i * UN_A + n, n % 2, mem)
        return mem

    def segment(layer, s, slot, mem):
        hs = jnp.concatenate([mem, h[slot]], axis=0)
        nxt = rows_of(jnp.minimum(s + 1, n_seg - 1))
        h[1 - slot] = _layernorm(nxt[...].astype(F32))
        fold(jnp.maximum(s - 1, 0))
        row, col = _iota((L, L), 0), _iota((L, L), 1)
        mask = (row < M) | (row >= col)

        tail = pl.ds(pl.multiple_of((s % per * RADIX + s // per) * 8, 8), 8)

        def linear(g):
            heads = range(g * GROUP, (g + 1) * GROUP)
            wg = _unpack([w[j] if g < PRE else w1[j - PRE * GROUP]
                          for j in heads])
            if layer > 0 or g >= PRE:
                return _dot(hs, wg)
            done = jnp.concatenate([pre[j, tail, :] for j in heads], axis=1)
            return jnp.concatenate([_dot(hs[:L - 8], wg), done], axis=0)

        def project(g):
            q, k, v = [linear(t * n_grp + g) for t in range(3)]
            return q, k.astype(BF16), v.astype(BF16)

        def probs(q, k):
            out = []
            for j in range(GROUP):
                c = slice(j * Dh, (j + 1) * Dh)
                sc = jnp.where(mask, _dot_t(q[:, c], k[:, c]) * scale, NEG)
                e = jnp.exp(sc - jnp.max(sc, axis=-1, keepdims=True))
                out.append((e, pltpu.reciprocal(
                    jnp.sum(e, axis=-1, keepdims=True), approx=True)))
            return out

        def attend(ps, v):
            return jnp.concatenate(
                [_dot(e, v[:, j * Dh:(j + 1) * Dh]) * inv
                 for j, (e, inv) in enumerate(ps)], axis=1)

        qkv, ps, os_ = {}, {}, {}
        acc = None
        for t in range(n_grp + 3):
            if t < n_grp:
                qkv[t] = project(t)
            if 0 <= t - 1 < n_grp:
                ps[t - 1] = probs(qkv[t - 1][0], qkv[t - 1][1])
            if 0 <= t - 2 < n_grp:
                os_[t - 2] = attend(ps[t - 2], qkv[t - 2][2])
            if 0 <= t - 3 < n_grp:
                g = t - 3
                y = _dot(os_[g], _unpack(
                    [wo[c, g * gw // 2:(g + 1) * gw // 2, :]
                     for c in range(D // LANES)]))
                acc = y if acc is None else acc + y
        cur = rows_of(s)
        cur[...] = (cur[...].astype(F32) + acc[M:]).astype(BF16)
        return acc[:M]

    def spectral(layer):
        fold(n_seg - 1)

        hr = RADIX // 2
        for i in range(0, nb, ch):
            for odd in range(2):
                halves = []
                for o in range(i, i + ch, 8):
                    lo, hi = fx[:hr, o:o + 8, :], fx[hr:, o:o + 8, :]
                    halves.append((lo - hi if odd else lo + hi)
                                  .reshape(hr * 8, D))
                t = tiles(jnp.concatenate(halves, axis=0))
                for c, p in enumerate([t[:1], t[1:3], t[3:]]):
                    k = len(p) * kt
                    re, im = tiles(_dot(
                        jnp.concatenate(p, axis=1),
                        _unpack([fd[c, 0, :k], fd[c, 1, :k]])))

                    def term(n, a):
                        r = slice((n * hr + a) * 8, (n * hr + a + 1) * 8)
                        return _twiddle((re[r], im[r]), a * odd, RADIX, -1)

                    out = [_fft([functools.partial(term, n, a)
                                 for a in range(hr)], -1)
                           for n in range(ch // 8)]
                    for f in range(hr):
                        for half in range(2):
                            v = jnp.concatenate([q[f][half] for q in out], 0)
                            r = pl.ds((i + half * nb) // 2, ch // 2)
                            ub[2 * f + odd, c, r, :] = pltpu.bitcast(
                                v.astype(BF16), jnp.uint32)

        zs = {}
        for t in range(hr + 1):
            for f1 in (t, t + hr) if t < hr else ():
                y = _dot(_unpack([fs[f1, 0]]),
                         _unpack([ub[f1, c] for c in range(nc)]))
                yr, yi = y[:nb], y[nb:]
                wr, wi = filt[f1, :, :P], filt[f1, :, P:]
                zs[f1] = jnp.concatenate(
                    [yr * wr - yi * wi, yr * wi + yi * wr], 0).astype(BF16)
            if t:
                f = t - 1
                lo, hi = [_dot(_unpack([ism[f1, 0]]), zs.pop(f1))
                          for f1 in (f, f + hr)]
                ev, od = lo + hi, lo - hi
                od = _twiddle((od[:nb], od[nb:]), f, RADIX, 1)
                for f1, (re, im) in ((f, (ev[:nb], ev[nb:])), (f + hr, od)):
                    for c, v in enumerate(tiles(re) + tiles(im)):
                        u[c, f1 * nb:(f1 + 1) * nb, :] = v

        for i in range(0, nb, ch):
            r = pl.ds(i, ch)
            for odd in range(2):
                ys = []
                for o in range(i, i + ch, 8):
                    def term(c, f):
                        rows = pl.ds((f + odd * hr) * nb + o, 8)
                        return u[c, rows, :], u[nc + c, rows, :]

                    g = []
                    for c in range(nc):
                        out = _fft([functools.partial(term, c, f)
                                    for f in range(hr)], 1)
                        z = jnp.concatenate(
                            [jnp.concatenate(v, axis=1) for v in out], axis=0)
                        g += tiles(_dot(z, _unpack(
                            [idm[c, n] for n in range(2 if c else 1)])))
                    g0, g1r, g1i, g2r, g2i = g
                    a1 = g0 + c1 * g1r + c2 * g2r
                    a2 = g0 + c2 * g1r + c1 * g2r
                    b1, b2 = s1 * g1i + s2 * g2i, s2 * g1i - s1 * g2i
                    ys.append(jnp.concatenate(
                        [g0 + g1r + g2r, a1 - b1, a2 - b2, a2 + b2, a1 + b1],
                        axis=1))
                for a in range(hr):
                    y = jnp.concatenate([v[a * 8:a * 8 + 8] for v in ys], 0)
                    x[2 * a + odd, r, :] = (
                        x[2 * a + odd, r, :].astype(F32) + y).astype(BF16)

            @pl.when(layer == 1)
            def _():
                pltpu.make_async_copy(x.at[:, r, :], o_hbm.at[:, r, :],
                                      out_sem).start()

    @pl.loop(0, 2)
    def _(layer):
        h[0] = _layernorm(x[0, :seg, :].astype(F32))
        for n in range(2):
            @pl.when(layer == n)
            def _():
                jax.lax.fori_loop(0, n_seg // UN_A,
                                  functools.partial(segments, n),
                                  memb[...].astype(F32))
                if n == 0:
                    for cp in cp_dft:
                        cp.wait()

        spectral(layer)

    pltpu.make_async_copy(x, o_hbm, out_sem).wait()


@functools.partial(jax.jit, static_argnames=("A_seg_len",))
def pallas_interleave_layers__memory_aug_recurrent_mem_tr__spectral_gfnet__prompt_kernel(
    A_x, A_mem0, A_Wq, A_Wk, A_Wv, A_Wo, A_seg_len, B_x, B_w_r, B_w_i,
):
    del B_x
    B, S, D = A_x.shape
    _, H, Dh = A_Wq.shape
    M = A_mem0.shape[1]
    assert B == 1 and Dh == LANES and D == 5 * LANES
    consts = _dft_constants(S, D)
    n_seg = S // A_seg_len
    per = n_seg // RADIX
    args = [A_x.reshape(RADIX, S // RADIX, D), A_mem0.reshape(M, D),
            A_Wq.reshape(D // 2, 2 * H, Dh), A_Wk.reshape(D // 2, 2 * H, Dh),
            A_Wv.reshape(D // 2, 2 * H, Dh), A_Wo.reshape(H * Dh, D),
            B_w_r.T, B_w_i.T] + consts
    u32 = jnp.uint32
    out = pl.pallas_call(
        functools.partial(_kernel, S=S, D=D, H=H, Dh=Dh, M=M, seg=A_seg_len),
        out_shape=jax.ShapeDtypeStruct((RADIX, S // RADIX, D), BF16),
        in_specs=[pl.BlockSpec(memory_space=pltpu.HBM)] * len(args),
        out_specs=pl.BlockSpec(memory_space=pltpu.HBM),
        scratch_shapes=[
            pltpu.VMEM((RADIX, S // RADIX, D), BF16),
            pltpu.VMEM((M, D), BF16),
            pltpu.VMEM((4, D // 2 * (H // 4), Dh), u32),
            pltpu.VMEM((4, D // 2 * (H // 2 + 8), Dh), u32),
            pltpu.VMEM((PRE * GROUP, D // 2, Dh), u32),
            pltpu.VMEM((3 * H - PRE * GROUP, D // 2, Dh), u32),
            pltpu.VMEM((D // LANES, H * Dh // 2, LANES), u32),
            pltpu.VMEM(B_w_r.shape[::-1], BF16),
            pltpu.VMEM(B_w_i.shape[::-1], BF16),
        ] + [pltpu.VMEM(c.shape, u32) for c in consts] + [
            pltpu.VMEM((S // LANES // 2, 3 * LANES, LANES), F32),
            pltpu.VMEM((per, RADIX, 8, D), BF16),
            pltpu.VMEM((n_seg * 4, D), u32),
            pltpu.VMEM((PRE * GROUP, n_seg * 8, Dh), F32),
            pltpu.VMEM((2, A_seg_len, D), F32),
            pltpu.VMEM((RADIX, S // RADIX, D), F32),
            pltpu.VMEM((RADIX, 3, S // RADIX, LANES), u32),
            pltpu.VMEM((6, S // RADIX * (RADIX + 8), LANES), F32),
            pltpu.VMEM((RADIX, S // RADIX, 6 * LANES), F32),
            pltpu.SemaphoreType.DMA((17 + D // LANES + per,)),
            pltpu.SemaphoreType.DMA(()),
        ],
        compiler_params=pltpu.CompilerParams(vmem_limit_bytes=110 * 2 ** 20),
    )(*args)
    return out.reshape(B, S, D)
```

```python
import functools
import math

import jax
import jax.numpy as jnp
import numpy as np
import jax.experimental.pallas as pl
import jax.experimental.pallas.tpu as pltpu

F32 = jnp.float32
BF16 = jnp.bfloat16
LANES = 128
RADIX = 32
GROUP = 4
SPLIT = 4
PRE = 14
UN_A = 2
EPS = 1e-5
NEG = -1000000000.0


def _pack(a):
    bits = a.astype(np.float32).astype(BF16).view(np.uint16).astype(np.uint32)
    words = bits[..., 0::2, :] | (bits[..., 1::2, :] << 16)
    words = words.reshape(words.shape[:-1] + (-1, LANES))
    return np.ascontiguousarray(np.swapaxes(words, -2, -3))


def _dft_constants(S, D):
    j = np.arange(LANES)
    b = j[:, None]
    fwd_d, inv_d = [], []
    for k1 in range(3):
        k = np.where(j < 64, k1 + 5 * j, D - (5 - k1) - 5 * (j - 64))
        wgt = np.full((LANES,), 2.0)
        if k1 == 0:
            k = 5 * j
            wgt = np.where(j < 64, 2.0, 0.0)
            wgt[0] = wgt[64] = 1.0
        ang = 2.0 * np.pi * ((b * k) % D) / D
        c, s = np.cos(ang), np.sin(ang)
        s[:, (2 * k) % D == 0] = 0.0
        m = np.block([[c, -s], [s, c]])
        fwd_d.append(m)
        inv_d.append(m.T * np.tile(wgt, 2)[:, None] / D)
    j = np.arange(S // RADIX)
    f = np.arange(RADIX)[:, None, None] + RADIX * j[None, :, None]
    ang = 2.0 * np.pi * ((j[None, None, :] * f) % S) / S
    c, s = np.cos(ang), np.sin(ang)
    fwd_s = np.concatenate([np.concatenate([c, s], 2),
                            np.concatenate([-s, c], 2)], 1)
    inv_s = np.swapaxes(fwd_s, 1, 2) / S
    return [_pack(a) for a in (np.stack(fwd_d), np.stack(inv_d), fwd_s, inv_s)]


def _twiddle(v, j, n, sign):
    pr, pi = v
    c = math.cos(2 * math.pi * j / n)
    s = sign * math.sin(2 * math.pi * j / n)
    if j == 0:
        return v
    if 4 * j == n:
        return (-pi, pr) if sign > 0 else (pi, -pr)
    if 8 * j % n == 0:
        return (((pr - pi) * c, (pr + pi) * c) if c * s > 0 else
                ((pr + pi) * c, (pi - pr) * c))
    return pr * c - pi * s, pr * s + pi * c


def _fft(vals, sign):
    n = len(vals)
    if n == 1:
        return [vals[0]()]
    ev, od = _fft(vals[0::2], sign), _fft(vals[1::2], sign)
    lo, hi = [], []
    for j in range(n // 2):
        er, ei = ev[j]
        if 4 * j == n:
            pr, pi = od[j]
            a, b = (er - pi, ei + pr), (er + pi, ei - pr)
            lo.append(a if sign > 0 else b)
            hi.append(b if sign > 0 else a)
        else:
            pr, pi = _twiddle(od[j], j, n, sign)
            lo.append((er + pr, ei + pi))
            hi.append((er - pr, ei - pi))
    return lo + hi


def _dot(a, b):
    return jax.lax.dot_general(a, b, (((1,), (0,)), ((), ())),
                               preferred_element_type=F32)


def _dot_t(a, b):
    return jax.lax.dot_general(a, b, (((1,), (1,)), ((), ())),
                               preferred_element_type=F32)


def _unpack(tiles):
    return pltpu.bitcast(jnp.concatenate(tiles, axis=1), BF16)


def _layernorm(x):
    xc = x - jnp.mean(x, axis=-1, keepdims=True)
    var = jnp.mean(xc * xc, axis=-1, keepdims=True)
    return xc * jax.lax.rsqrt(var + EPS)


def _iota(shape, axis):
    return jax.lax.broadcasted_iota(jnp.int32, shape, axis)


def _kernel(x_hbm, mem_hbm, wq_hbm, wk_hbm, wv_hbm, wo_hbm, wr_hbm, wi_hbm,
            fd_hbm, id_hbm, fs_hbm, is_hbm, o_hbm,
            x, memb, stage_q, stage, w, w1, wo, wrb, wib, fd, idm, fs, ism,
            tmp, xt, ht, pre, h, fx, ub, u, filt, sems, out_sem, *, S, D, H, Dh, M, seg):
    L = M + seg
    n_seg = S // seg
    nb = S // RADIX
    nc = 3
    P = nc * LANES
    Df = wrb.shape[0]
    scale = Dh ** -0.5

    started = []

    def fetch(src, dst):
        cp = pltpu.make_async_copy(src, dst, sems.at[len(started)])
        cp.start()
        started.append(cp)
        return cp

    per = nb // seg

    def fetch_w(src, buf, slot, lo, n):
        pitch = buf.shape[1] // (D // 2)
        return [fetch(
            src.bitcast(jnp.uint32).at[:, pl.ds(par * H // 2 + lo, n)],
            buf.at[2 * slot + par, pl.ds(0, D // 2 * pitch)]
            .reshape(D // 2, pitch, Dh).at[:, pl.ds(0, n)])
            for par in range(2)]

    cp_tail = [fetch(x_hbm.at[:, pl.ds((n + 1) * seg - 8, 8)], xt.at[n])
               for n in range(per)]
    cp_q = [fetch_w(wq_hbm, stage_q, n, n * H // 4, H // 4) for n in range(2)]
    cp_filt = [fetch(wr_hbm, wrb), fetch(wi_hbm, wib)]
    cp_k = fetch_w(wk_hbm, stage, 0, 0, H // 2)
    cp_v = fetch_w(wv_hbm, stage, 1, 0, H // 2)
    n0 = pl.cdiv((UN_A + 1) * seg, nb)
    first = [fetch(mem_hbm, memb), fetch(x_hbm.at[:n0], x.at[:n0])]
    first += [fetch(wo_hbm.bitcast(jnp.uint32).at[:, pl.ds(c * LANES, LANES)],
                    wo.at[c])
              for c in range(D // LANES)]

    n_part = tmp.shape[0]
    gap = RADIX + 8

    def transpose_filter(i):
        for n in range(n_part):
            blk = i * (n_part // 2) + n // 2
            r = pl.ds(pl.multiple_of(blk * LANES, LANES), LANES)
            tmp[n] = jnp.concatenate(
                [(wrb, wib)[n % 2][:, r].astype(F32),
                 jnp.zeros((P - Df, LANES), F32)], 0)
            yield
            for c in range(nc):
                v = jnp.concatenate(
                    [tmp[n, pl.ds(c, 64 if c else 72, stride=5), :],
                     tmp[n, pl.ds(5 - c, 64, stride=5), :] if c
                     else jnp.zeros((56, LANES), F32)], axis=0).T
                for m in range(LANES // RADIX):
                    o = pl.multiple_of((blk * (LANES // RADIX) + m) * gap, 8)
                    u[n % 2 * nc + c, pl.ds(o, RADIX), :] = (
                        v[m * RADIX:(m + 1) * RADIX])
                yield

    def gather_filter(i):
        for n in range(n_part):
            f1 = i * n_part + n
            pos = _iota((nb, nb), 0) + _iota((nb, nb), 1) + jnp.minimum(f1, 1)
            flip = jnp.where((pos == 0) | (pos == nb), 1.0, 0.0)
            neg = pl.ds((RADIX - f1) % RADIX, nb, stride=gap)
            mixed = [c for c in range(2 * nc) if c % nc]
            m = _dot(flip, jnp.concatenate(
                [u[c, neg, :] for c in mixed], axis=1).astype(BF16))
            yield
            yield
            for c in range(2 * nc):
                v = u[c, pl.ds(f1, nb, stride=gap), :]
                if c % nc:
                    o = mixed.index(c) * LANES
                    mc = m[:, o:o + LANES]
                    v = jnp.where(_iota((nb, LANES), 1) < 64, v,
                                  mc if c < nc else -mc)
                filt[f1, :, c * LANES:(c + 1) * LANES] = v
                if c % 2:
                    yield

    n_grp = H // GROUP
    kt = LANES // 2

    def regroup(pair, is_q, dst, base):
        buf, n, q = ((stage_q, H // 4, pair) if is_q else
                     (stage, H // 2, pair - H // 2))
        pitch = buf.shape[1] // (D // 2)
        for k in range(0, D // 2, kt):
            j = pl.ds(q % n + k * pitch, kt, stride=pitch)
            a, b = [buf[q // n * 2 + par, j, :] for par in range(2)]
            even = (a & jnp.uint32(0xFFFF)) | (b << 16)
            odd = (a >> 16) | (b & jnp.uint32(0xFFFF0000))
            dst[2 * pair - base, k:k + kt] = even
            dst[2 * pair - base + 1, k:k + kt] = odd
            yield [even, odd]

    def regroup_rest(i):
        cnt, rem = divmod((3 * H - PRE * GROUP) // 2, PRE - 12)
        assert rem == 0
        for n in range(cnt):
            yield from regroup(PRE * GROUP // 2 + i * cnt + n, False, w1,
                               PRE * GROUP)

    def project_tails(lo, hi, waits, job=lambda i: iter(())):
        for cp in waits:
            cp.wait()

        @pl.loop(0, hi - lo)
        def _(i):
            fresh = [regroup((lo + i) * (GROUP // 2) + n, lo < n_grp, w, 0)
                     for n in range(GROUP // 2)]
            heads = [(lo + i) * GROUP + j for j in range(GROUP)]
            rows = n_seg * 8 // SPLIT
            extra = job(i)
            for n in range(SPLIT):
                y = 0.0
                for k in range(0, D // 2, kt):
                    wk = (sum((next(f) for f in fresh), []) if n == 0 else
                          [w[j, k:k + kt] for j in heads])
                    lhs = ht[n * rows // 2:(n + 1) * rows // 2,
                             2 * k:2 * k + LANES]
                    y += _dot(_unpack([lhs]), _unpack(wk))
                    for _ in range(n_part // SPLIT):
                        next(extra, None)
                for j in range(GROUP):
                    pre[heads[j], n * rows:(n + 1) * rows] = (
                        y[:, j * Dh:(j + 1) * Dh])
            for _ in extra:
                pass

    for cp in cp_tail:
        cp.wait()
    ht[...] = pltpu.bitcast(_layernorm(
        xt[...].astype(F32).reshape(n_seg * 8, D)).astype(BF16), jnp.uint32)
    project_tails(0, 4, cp_q[0])
    project_tails(4, 8, cp_q[1] + cp_filt, transpose_filter)
    project_tails(8, 12, cp_k, gather_filter)
    project_tails(12, PRE, cp_v, regroup_rest)

    for cp in first:
        cp.wait()
    rest = pl.ds(n0, RADIX - n0)
    cp_x = fetch(x_hbm.at[rest], x.at[rest])
    cp_dft = [fetch(fd_hbm, fd), fetch(fs_hbm, fs), fetch(is_hbm, ism),
              fetch(id_hbm, idm)]

    gw = GROUP * Dh

    c1, c2 = math.cos(0.4 * math.pi), math.cos(0.8 * math.pi)
    s1, s2 = math.sin(0.4 * math.pi), math.sin(0.8 * math.pi)
    ch = 16

    def tiles(v):
        return [v[:, c:c + LANES] for c in range(0, v.shape[1], LANES)]

    def fold(s):
        t = tiles(_layernorm(rows_of(s)[...].astype(F32)))
        a1, a2, d1, d2 = t[1] + t[4], t[2] + t[3], t[4] - t[1], t[3] - t[2]
        rows_of(s, fx)[...] = jnp.concatenate(
            [t[0] + a1 + a2,
             t[0] + c1 * a1 + c2 * a2, s1 * d1 + s2 * d2,
             t[0] + c2 * a1 + c1 * a2, s2 * d1 - s1 * d2], axis=1)

    def rows_of(s, ref=x):
        return ref.at[s // per, pl.ds(pl.multiple_of(s % per * seg, seg), seg)]

    def segments(layer, i, mem):
        if layer == 0:
            pl.when(i == 1)(cp_x.wait)
        for n in range(UN_A):
            mem = segment(layer, i * UN_A + n, n % 2, mem)
        return mem

    def segment(layer, s, slot, mem):
        hs = jnp.concatenate([mem, h[slot]], axis=0)
        nxt = rows_of(jnp.minimum(s + 1, n_seg - 1))
        h[1 - slot] = _layernorm(nxt[...].astype(F32))
        fold(jnp.maximum(s - 1, 0))
        row, col = _iota((L, L), 0), _iota((L, L), 1)
        mask = (row < M) | (row >= col)

        tail = pl.ds(pl.multiple_of((s % per * RADIX + s // per) * 8, 8), 8)

        def linear(g):
            heads = range(g * GROUP, (g + 1) * GROUP)
            wg = _unpack([w[j] if g < PRE else w1[j - PRE * GROUP]
                          for j in heads])
            if layer > 0 or g >= PRE:
                return _dot(hs, wg)
            done = jnp.concatenate([pre[j, tail, :] for j in heads], axis=1)
            return jnp.concatenate([_dot(hs[:L - 8], wg), done], axis=0)

        def project(g):
            q, k, v = [linear(t * n_grp + g) for t in range(3)]
            return q, k.astype(BF16), v.astype(BF16)

        def probs(q, k):
            out = []
            for j in range(GROUP):
                c = slice(j * Dh, (j + 1) * Dh)
                sc = jnp.where(mask, _dot_t(q[:, c], k[:, c]) * scale, NEG)
                e = jnp.exp(sc - jnp.max(sc, axis=-1, keepdims=True))
                out.append((e, pltpu.reciprocal(
                    jnp.sum(e, axis=-1, keepdims=True), full_range=False)))
            return out

        def attend(ps, v):
            return jnp.concatenate(
                [_dot(e, v[:, j * Dh:(j + 1) * Dh]) * inv
                 for j, (e, inv) in enumerate(ps)], axis=1)

        qkv, ps, os_ = {}, {}, {}
        acc = None
        for t in range(n_grp + 3):
            if t < n_grp:
                qkv[t] = project(t)
            if 0 <= t - 1 < n_grp:
                ps[t - 1] = probs(qkv[t - 1][0], qkv[t - 1][1])
            if 0 <= t - 2 < n_grp:
                os_[t - 2] = attend(ps[t - 2], qkv[t - 2][2])
            if 0 <= t - 3 < n_grp:
                g = t - 3
                y = _dot(os_[g], _unpack(
                    [wo[c, g * gw // 2:(g + 1) * gw // 2, :]
                     for c in range(D // LANES)]))
                acc = y if acc is None else acc + y
        cur = rows_of(s)
        cur[...] = (cur[...].astype(F32) + acc[M:]).astype(BF16)
        return acc[:M]

    def spectral(layer):
        fold(n_seg - 1)

        hr = RADIX // 2
        for i in range(0, nb, ch):
            for odd in range(2):
                halves = []
                for o in range(i, i + ch, 8):
                    lo, hi = fx[:hr, o:o + 8, :], fx[hr:, o:o + 8, :]
                    halves.append((lo - hi if odd else lo + hi)
                                  .reshape(hr * 8, D))
                t = tiles(jnp.concatenate(halves, axis=0))
                for c, p in enumerate([t[:1], t[1:3], t[3:]]):
                    k = len(p) * kt
                    re, im = tiles(_dot(
                        jnp.concatenate(p, axis=1),
                        _unpack([fd[c, 0, :k], fd[c, 1, :k]])))

                    def term(n, a):
                        r = slice((n * hr + a) * 8, (n * hr + a + 1) * 8)
                        return _twiddle((re[r], im[r]), a * odd, RADIX, -1)

                    out = [_fft([functools.partial(term, n, a)
                                 for a in range(hr)], -1)
                           for n in range(ch // 8)]
                    for f in range(hr):
                        for half in range(2):
                            v = jnp.concatenate([q[f][half] for q in out], 0)
                            r = pl.ds((i + half * nb) // 2, ch // 2)
                            ub[2 * f + odd, c, r, :] = pltpu.bitcast(
                                v.astype(BF16), jnp.uint32)

        zs = {}
        for t in range(hr + 1):
            for f1 in (t, t + hr) if t < hr else ():
                y = _dot(_unpack([fs[f1, 0]]),
                         _unpack([ub[f1, c] for c in range(nc)]))
                yr, yi = y[:nb], y[nb:]
                wr, wi = filt[f1, :, :P], filt[f1, :, P:]
                zs[f1] = jnp.concatenate(
                    [yr * wr - yi * wi, yr * wi + yi * wr], 0).astype(BF16)
            if t:
                f = t - 1
                lo, hi = [_dot(_unpack([ism[f1, 0]]), zs.pop(f1))
                          for f1 in (f, f + hr)]
                ev, od = lo + hi, lo - hi
                od = _twiddle((od[:nb], od[nb:]), f, RADIX, 1)
                for f1, (re, im) in ((f, (ev[:nb], ev[nb:])), (f + hr, od)):
                    for c, v in enumerate(tiles(re) + tiles(im)):
                        u[c, f1 * nb:(f1 + 1) * nb, :] = v

        for i in range(0, nb, ch):
            r = pl.ds(i, ch)
            for odd in range(2):
                ys = []
                for o in range(i, i + ch, 8):
                    def term(c, f):
                        rows = pl.ds((f + odd * hr) * nb + o, 8)
                        return u[c, rows, :], u[nc + c, rows, :]

                    g = []
                    for c in range(nc):
                        out = _fft([functools.partial(term, c, f)
                                    for f in range(hr)], 1)
                        z = jnp.concatenate(
                            [jnp.concatenate(v, axis=1) for v in out], axis=0)
                        g += tiles(_dot(z, _unpack(
                            [idm[c, n] for n in range(2 if c else 1)])))
                    g0, g1r, g1i, g2r, g2i = g
                    a1 = g0 + c1 * g1r + c2 * g2r
                    a2 = g0 + c2 * g1r + c1 * g2r
                    b1, b2 = s1 * g1i + s2 * g2i, s2 * g1i - s1 * g2i
                    ys.append(jnp.concatenate(
                        [g0 + g1r + g2r, a1 - b1, a2 - b2, a2 + b2, a1 + b1],
                        axis=1))
                for a in range(hr):
                    y = jnp.concatenate([v[a * 8:a * 8 + 8] for v in ys], 0)
                    x[2 * a + odd, r, :] = (
                        x[2 * a + odd, r, :].astype(F32) + y).astype(BF16)

            @pl.when(layer == 1)
            def _():
                pltpu.make_async_copy(x.at[:, r, :], o_hbm.at[:, r, :],
                                      out_sem).start()

    @pl.loop(0, 2)
    def _(layer):
        h[0] = _layernorm(x[0, :seg, :].astype(F32))
        for n in range(2):
            @pl.when(layer == n)
            def _():
                jax.lax.fori_loop(0, n_seg // UN_A,
                                  functools.partial(segments, n),
                                  memb[...].astype(F32))
                if n == 0:
                    for cp in cp_dft:
                        cp.wait()

        spectral(layer)

    pltpu.make_async_copy(x, o_hbm, out_sem).wait()


@functools.partial(jax.jit, static_argnames=("A_seg_len",))
def pallas_interleave_layers__memory_aug_recurrent_mem_tr__spectral_gfnet__prompt_kernel(
    A_x, A_mem0, A_Wq, A_Wk, A_Wv, A_Wo, A_seg_len, B_x, B_w_r, B_w_i,
):
    del B_x
    B, S, D = A_x.shape
    _, H, Dh = A_Wq.shape
    M = A_mem0.shape[1]
    assert (B, S, D, H, Dh, M, A_seg_len) == (1, 2048, 640, 32, 128, 8, 32)
    consts = _dft_constants(S, D)
    n_seg = S // A_seg_len
    per = n_seg // RADIX
    args = [A_x.reshape(RADIX, S // RADIX, D), A_mem0.reshape(M, D),
            A_Wq.reshape(D // 2, 2 * H, Dh), A_Wk.reshape(D // 2, 2 * H, Dh),
            A_Wv.reshape(D // 2, 2 * H, Dh), A_Wo.reshape(H * Dh, D),
            B_w_r.T, B_w_i.T] + consts
    u32 = jnp.uint32
    out = pl.pallas_call(
        functools.partial(_kernel, S=S, D=D, H=H, Dh=Dh, M=M, seg=A_seg_len),
        out_shape=jax.ShapeDtypeStruct((RADIX, S // RADIX, D), BF16),
        in_specs=[pl.BlockSpec(memory_space=pltpu.HBM)] * len(args),
        out_specs=pl.BlockSpec(memory_space=pltpu.HBM),
        scratch_shapes=[
            pltpu.VMEM((RADIX, S // RADIX, D), BF16),
            pltpu.VMEM((M, D), BF16),
            pltpu.VMEM((4, D // 2 * (H // 4) + 8, Dh), u32),
            pltpu.VMEM((4, D // 2 * (H // 2 + 8) + 16, Dh), u32),
            pltpu.VMEM((PRE * GROUP, D // 2, Dh), u32),
            pltpu.VMEM((3 * H - PRE * GROUP, D // 2, Dh), u32),
            pltpu.VMEM((D // LANES, H * Dh // 2, LANES), u32),
            pltpu.VMEM(B_w_r.shape[::-1], BF16),
            pltpu.VMEM(B_w_i.shape[::-1], BF16),
        ] + [pltpu.VMEM(c.shape, u32) for c in consts] + [
            pltpu.VMEM((S // LANES // 2, 3 * LANES, LANES), F32),
            pltpu.VMEM((per, RADIX, 8, D), BF16),
            pltpu.VMEM((n_seg * 4, D), u32),
            pltpu.VMEM((PRE * GROUP, n_seg * 8, Dh), F32),
            pltpu.VMEM((2, A_seg_len, D), F32),
            pltpu.VMEM((RADIX, S // RADIX, D), F32),
            pltpu.VMEM((RADIX, 3, S // RADIX, LANES), u32),
            pltpu.VMEM((6, (S // RADIX + 1) * (RADIX + 8), LANES), F32),
            pltpu.VMEM((RADIX, S // RADIX, 6 * LANES), F32),
            pltpu.SemaphoreType.DMA((17 + D // LANES + per,)),
            pltpu.SemaphoreType.DMA(()),
        ],
        compiler_params=pltpu.CompilerParams(vmem_limit_bytes=110 * 2 ** 20),
    )(*args)
    return out.reshape(B, S, D)
```
